```python
import os as _os
_os.environ.setdefault('JAX_PLATFORMS', 'cpu')
import jax
import jax.numpy as jnp

def _softmax(x, axis=-1):
    return jax.nn.softmax(x, axis=axis)

def _gelu(x):
    return jax.nn.gelu(x, approximate=True)

def _silu(x):
    return jax.nn.silu(x)

def _sigmoid(x):
    return jax.nn.sigmoid(x)

def _layernorm(x, axis=-1, eps=1e-05):
    m = jnp.mean(x, axis=axis, keepdims=True)
    v = jnp.var(x, axis=axis, keepdims=True)
    return (x - m) / jnp.sqrt(v + eps)

def _scatter_add(tgt, idx, src, axis=0):
    return tgt.at[idx].add(src)

def _segment_sum(src, seg, n):
    return jax.ops.segment_sum(src, seg, n)

class _Rng:

    def __init__(self, key):
        self._k = key

    def _next(self):
        self._k, sub = jax.random.split(self._k)
        return sub

    def normal(self, shape):
        return jax.random.normal(self._next(), shape, dtype=jnp.bfloat16)

    def randint(self, lo, hi, shape):
        return jax.random.randint(self._next(), shape, lo, hi, dtype=jnp.int32)

    def uniform(self, shape, lo=0.0, hi=1.0):
        return jax.random.uniform(self._next(), shape, jnp.bfloat16, lo, hi)

    def permutation(self, n):
        return jax.random.permutation(self._next(), n)
kernel_name = 'interleave_layers__ssm_conv_h3__mixer_gmlp__prompt'

def setup_inputs():
    _rng = _Rng(jax.random.key(int.from_bytes(__import__("os").urandom(4), "little")))
    _w = lambda a: (lambda t: t.astype(jnp.bfloat16) if jnp.issubdtype(t.dtype, jnp.floating) else t)(jnp.asarray(a))

    def _A_setup():
        B, S, D = (1, 2048, 1024)
        ks = 4
        return {'q': _w((lambda *s: _rng.normal(s) * 0.05)(B, S, D)), 'k': _w((lambda *s: _rng.normal(s) * 1.6)(B, S, D)), 'v': _w((lambda *s: _rng.normal(s) * 1.6)(B, S, D)), 'shift_k': _w((lambda *s: _rng.normal(s) * 1.6)(D, ks) * 0.5), 'ssm_k': _w((lambda *s: _rng.normal(s) * 1.6)(D, S) * (1.0 / S ** 0.5)), 'ssm_D': _w((lambda *s: _rng.normal(s) * 1.6)(D))}
    _A_in = _A_setup()

    def _B_setup():
        B, S, D, F = (1, 2048, 1024, 3584)
        Fh = F // 2
        return {'x': _w((lambda *s: _rng.normal(s) * 0.05)(B, S, D)), 'w_in': _w((lambda *s: _rng.normal(s) * 0.8)(D, 2 * Fh)), 'w_sp': _w(0.01 * (lambda *s: _rng.normal(s) * 0.8)(S, S)), 'b_sp': _w(1.0 + 0.01 * (lambda *s: _rng.normal(s) * 0.2)(S)), 'w_out': _w((lambda *s: _rng.normal(s) * 0.2)(Fh, D))}
    _B_in = _B_setup()
    return {'A_q': _A_in['q'], 'A_k': _A_in['k'], 'A_v': _A_in['v'], 'A_shift_k': _A_in['shift_k'], 'A_ssm_k': _A_in['ssm_k'], 'A_ssm_D': _A_in['ssm_D'], 'B_x': _B_in['x'], 'B_w_in': _B_in['w_in'], 'B_w_sp': _B_in['w_sp'], 'B_b_sp': _B_in['b_sp'], 'B_w_out': _B_in['w_out']}

def reference(A_q, A_k, A_v, A_shift_k, A_ssm_k, A_ssm_D, B_x, B_w_in, B_w_sp, B_b_sp, B_w_out):

    def _A_ref(q, k, v, shift_k, ssm_k, ssm_D):
        B, S, D = q.shape
        ks = shift_k.shape[-1]
        k_pad = jnp.pad(k, ((0, 0), (ks - 1, 0), (0, 0)))
        k_shift = jnp.zeros_like(k)
        for t in range(ks):
            k_shift = k_shift + k_pad[:, t:t + S, :] * shift_k[:, ks - 1 - t][None, None, :]
        kv = k_shift * v
        L = 2 * S
        kv_pad = jnp.pad(kv, ((0, 0), (0, S), (0, 0)))
        kf_pad = jnp.pad(ssm_k, ((0, 0), (0, S)))
        kv_f = (lambda x, axes=(-2, -1): jnp.fft.rfft2(x.astype(jnp.float32), axes=axes))(kv_pad[:, None, :, :], axes=(1, 2))
        kf_f = (lambda x, axes=(-2, -1): jnp.fft.rfft2(x.astype(jnp.float32), axes=axes))(kf_pad[:, None, :], axes=(1, 2))
        kf_f = (lambda x, *d: x.transpose(*d))(kf_f, 1, 2, 0)
        y_f = kv_f * kf_f[None, :, :, :]
        y = (lambda x, s, axes=(-2, -1): jnp.fft.irfft2(x, s=s, axes=axes).astype(jnp.bfloat16))(y_f, (1, L), axes=(1, 2))[:, 0, :S, :]
        y = y + kv * ssm_D[None, None, :]
        return q * y

    def _B_ref(x, w_in, w_sp, b_sp, w_out):
        B, S, D = x.shape
        F = w_in.shape[-1]
        Fh = F // 2
        z = _gelu(jnp.einsum('bsd,df->bsf', x, w_in))
        z1 = z[..., :Fh].copy()
        z2 = _layernorm(z[..., Fh:], axis=-1)
        g = jnp.einsum('ts,bsf->btf', w_sp, z2) + b_sp[None, :, None]
        return jnp.einsum('bsf,fd->bsd', z1 * g, w_out)
    x = A_q
    x = x + _A_ref(_layernorm(x, axis=-1), A_k, A_v, A_shift_k, A_ssm_k, A_ssm_D)
    x = x + _B_ref(_layernorm(x, axis=-1), B_w_in, B_w_sp, B_b_sp, B_w_out)
    x = x + _A_ref(_layernorm(x, axis=-1), A_k, A_v, A_shift_k, A_ssm_k, A_ssm_D)
    x = x + _B_ref(_layernorm(x, axis=-1), B_w_in, B_w_sp, B_b_sp, B_w_out)
    return x
```

```python
import functools

import numpy as np
import jax
import jax.numpy as jnp
import jax.experimental.pallas as pl
import jax.experimental.pallas.tpu as pltpu

S = 2048
D = 1024
F = 3584
FH = F // 2
P = 128
NB = S // P
NG = D // 128
TM = 256
NR = S // TM
TN = 256
PR = 16
XC = F
RW = F + D
EPS = 1e-5

f32 = jnp.float32
bf16 = jnp.bfloat16


def _dft_constants():
    n = np.arange(P)
    k = np.concatenate([np.arange(0, P, 2), np.arange(1, P, 2)])
    ang = 2.0 * np.pi * np.outer(2 * k + 1, n) / (4 * P)
    fre, fim = np.cos(ang), -np.sin(ang)
    fu = np.concatenate([fre, fim], 0)
    fh = np.concatenate([fre, fim - fre, fre + fim], 0)
    g = np.concatenate([fre.T, fim.T], 0) / P
    return jnp.asarray(np.concatenate([fu, fh, g], 0), dtype=bf16)


def _ln(x):
    m = jnp.mean(x, axis=-1, keepdims=True)
    xc = x - m
    v = jnp.mean(xc * xc, axis=-1, keepdims=True)
    return xc * jax.lax.rsqrt(v + EPS)


def _gelu(z):
    c = 0.7978845608028654
    u = z * (c + (c * 0.044715) * (z * z))
    h = 0.5 * z
    return h + h * jnp.tanh(u)


def _dot(a, b):
    return jnp.dot(a, b, preferred_element_type=f32)


def _spread(work, n):
    return [work[(j * len(work)) // n:((j + 1) * len(work)) // n] for j in range(n)]


def _dot_nt(a, b):
    return jax.lax.dot_general(a, b, (((1,), (1,)), ((), ())), preferred_element_type=f32)


def _pack(x):
    return pltpu.bitcast(x, jnp.uint32)


def _unpack(x):
    return pltpu.bitcast(x, bf16)


_CONV_ORDER = "H0 lo0 H1 rh0 H2 ih0 lo1 U0 rh1 U1 ih1".split()
_NSUB = 4


def _kernel(q_hbm, k_hbm, v_hbm, shk_ref, hk_hbm, dv_ref, win_hbm, wsp_hbm, bsp_ref,
            wout_hbm, dft_ref, out_hbm,
            k_v, v_v, hk_v, win_v, wsp_v, wout_v, y_v, r1, r2, xnl, ml,
            w0, w1, kv0, kv1, kv2, kf_s, dft_p, bcol, sem_k, sem_v, sem_h, sem_w, sem_o):
    def grp_copies(g):
        cols = slice(g * 128, (g + 1) * 128)
        return (pltpu.make_async_copy(hk_hbm.at[cols, :], hk_v.at[cols, :], sem_h.at[g]),
                pltpu.make_async_copy(k_hbm.at[0, :, cols], k_v.at[:, cols], sem_k.at[g]),
                pltpu.make_async_copy(v_hbm.at[0, :, cols], v_v.at[:, cols], sem_v.at[g]))

    q_copy = pltpu.make_async_copy(q_hbm.at[0], r1.at[0:S, XC:XC + D], sem_w.at[0])
    win_copy = pltpu.make_async_copy(win_hbm, win_v, sem_w.at[1])
    wsp_copy = pltpu.make_async_copy(wsp_hbm, wsp_v, sem_w.at[2])
    wout_copy = pltpu.make_async_copy(wout_hbm, wout_v, sem_w.at[3])

    def out_copy(i):
        rows = pl.ds(pl.multiple_of(i * TM, TM), TM)
        return pltpu.make_async_copy(y_v.at[rows, :], out_hbm.at[0, rows, :], sem_o.at[i])

    for g in range(2):
        for c in grp_copies(g):
            c.start()

    ws, kvs = [w0, w1], [kv0, kv1, kv2]
    dft_p[...] = _pack(dft_ref[...])
    kf_s[0:8, :] = jnp.zeros((8, 128), f32)
    for w in ws:
        w[5, 0] = jnp.zeros((P, 128), f32)
        w[6, 0] = jnp.zeros((P, 128), f32)
    r1[S:S + TM, XC:XC + D] = jnp.zeros((TM, D), bf16)
    eye = (jax.lax.broadcasted_iota(jnp.int32, (128, 128), 0)
           == jax.lax.broadcasted_iota(jnp.int32, (128, 128), 1))
    brow = bsp_ref[...].astype(f32).reshape(1, S)
    for t in range(S // 128):
        row = jnp.broadcast_to(brow[:, t * 128:(t + 1) * 128], (128, 128))
        col = jnp.sum(jnp.where(eye, row, 0.0), axis=1, keepdims=True)
        bcol[t * 128:(t + 1) * 128, :] = jnp.broadcast_to(col, (128, 128))

    def dft(lo, n):
        return _unpack(dft_p[lo // 2:(lo + n) // 2, :])

    hp = P // 2

    def conv_iter(g, p):
        do_a, do_b, do_c = g < NG, 1 <= g <= NG, g >= 2
        ga, gc = g, g - 2
        wst, wld = ws[g % 2], ws[(g + 1) % 2]
        b0 = 2 * p
        r0 = pl.multiple_of(p * 2 * P, 2 * P)
        st = {}
        if do_a:
            cols = slice(ga * 128, (ga + 1) * 128)
            hd = []
            for j in range(2):
                hkb = hk_v[cols, pl.ds(pl.multiple_of(r0 + j * P, P), P)]
                hd.append(jnp.concatenate(
                    [_dot_nt(dft(2 * P, 192), hkb), _dot_nt(dft(2 * P + 192, 192), hkb)], 0))
        if do_c:
            cols = slice(gc * 128, (gc + 1) * 128)
            dvec = dv_ref[...].astype(f32).reshape(1, D)[:, cols]
            for j in range(2):
                cr, ci = wld[5, b0 + j + 1], wld[6, b0 + j + 1]
                pr, pi = wld[5, b0 + j], wld[6, b0 + j]
                a = jnp.concatenate([cr[:hp] - pi[:hp], cr[hp:] + pi[hp:]], 0).astype(bf16)
                b = jnp.concatenate([ci[:hp] + pr[:hp], ci[hp:] - pr[hp:]], 0).astype(bf16)
                yt = _dot(dft(5 * P, P), a) + _dot(dft(6 * P, P), b)
                rows = pl.ds(pl.multiple_of(r0 + j * P, P), P)
                kv = kvs[gc % 3][rows, :].astype(f32)
                y_v[rows, cols] = (yt + kv * dvec).astype(bf16)
        if do_a:
            cols = slice(ga * 128, (ga + 1) * 128)
            taps = shk_ref[:, cols].astype(f32)
            rows2 = pl.ds(r0, 2 * P)
            kf_s[pl.ds(pl.multiple_of(r0 + 8, 8), 2 * P), :] = k_v[rows2, cols].astype(f32)
            ks = kf_s[pl.ds(r0 + 8, 2 * P), :] * taps[0:1]
            for j in range(1, 4):
                ks = ks + kf_s[pl.ds(r0 + 8 - j, 2 * P), :] * taps[j:j + 1]
            kvs[ga % 3][rows2, :] = (ks * v_v[rows2, cols].astype(f32)).astype(bf16)
            ur, ui = [], []
            for j in range(2):
                kvb = kvs[ga % 3][pl.ds(pl.multiple_of(r0 + j * P, P), P), :]
                ur.append(_dot(dft(0, P), kvb))
                ui.append(_dot(dft(P, P), kvb))

        def ldu(which, b, r):
            if which == 2:
                return wld[0, b, r, :] + wld[1, b, r, :]
            return wld[which, b, r, :]

        def cv(hi, uw, r, ts):
            out, hs, us = {}, {}, {}
            for ub in ([range(0, 8)] if ts[0] == 0 else [range(8, 16), range(0, 8)]):
                for t in ts:
                    for b in ub:
                        d = t - b
                        if d < 0:
                            continue
                        if d not in hs:
                            hs[d] = wld[2 + hi, d, r, :]
                        if b not in us:
                            us[b] = ldu(uw, b, r)
                        term = hs[d] * us[b]
                        out[t] = term if t not in out else out[t] + term
            return out

        for o in _CONV_ORDER:
            if o[0] == "H":
                if do_a:
                    for j in range(2):
                        for half in range(2):
                            lo = half * 192 + int(o[1]) * 64
                            wst[2 + lo // P, b0 + j, lo % P:lo % P + 64, :] = hd[j][lo:lo + 64]
            elif o[0] == "U":
                if do_a:
                    rr = slice(int(o[1]) * hp, (int(o[1]) + 1) * hp)
                    for j in range(2):
                        wst[0, b0 + j, rr, :] = ur[j][rr]
                        wst[1, b0 + j, rr, :] = ui[j][rr]
            elif do_b:
                hh = int(o[2])
                r = pl.ds(pl.multiple_of(p * 16 + 8 * hh, 8), 8)
                ts = list(range(0, 8)) if o[:2] == "lo" else list(range(8, 16))
                key = (hh, ts[0])
                if key not in st:
                    st[key] = cv(0, 2, r, ts)
                s1 = st[key]
                if o[:2] in ("lo", "rh"):
                    s3 = cv(2, 1, r, ts)
                    for t in ts:
                        wst[5, t + 1, r, :] = s1[t] - s3[t]
                if o[:2] in ("lo", "ih"):
                    s2 = cv(1, 0, r, ts)
                    for t in ts:
                        wst[6, t + 1, r, :] = s1[t] + s2[t]

    for g in range(NG + 2):
        if g < NG:
            for c in grp_copies(g):
                c.wait()
        if g + 2 < NG:
            for c in grp_copies(g + 2):
                c.start()
        if g == 3:
            q_copy.start()
        if g == 5:
            win_copy.start()
        if g == NG + 1:
            wsp_copy.start()
            wout_copy.start()

        def conv_body(p, carry, g=g):
            for j in range(_NSUB):
                conv_iter(g, p * _NSUB + j)
            return carry

        jax.lax.fori_loop(0, NB // 2 // _NSUB, conv_body, 0)

    npc = TM // PR

    def rows_of(i, r0=0, nr=TM):
        return pl.ds(pl.multiple_of(i * TM + r0, PR), nr)

    def a_layer_piece(r, i, iy, ps, stage_c):
        if not ps:
            return
        rr = rows_of(i, ps[0] * PR, len(ps) * PR)
        ry = rows_of(iy, ps[0] * PR, len(ps) * PR)
        x = r[rr, XC:XC + D].astype(f32)
        x = x + _ln(x) * y_v[ry, :].astype(f32)
        r[rr, XC:XC + D] = x.astype(bf16)
        r[rr, stage_c:stage_c + D] = _ln(x).astype(bf16)

    def norm_piece(r, i, ps):
        if not ps:
            return
        rr = rows_of(i, ps[0] * PR, len(ps) * PR)
        r[rr, FH:F] = _ln(r[rr, FH:F].astype(f32)).astype(bf16)

    def z_chunk(r, i, c):
        cs = slice(c * TN, (c + 1) * TN)
        r[rows_of(i), cs] = _gelu(_dot(_unpack(xnl[...]), win_v[:, cs])).astype(bf16)

    def g_chunk(r, i, c):
        cs = slice(c * TN, (c + 1) * TN)
        rr = rows_of(i)
        gg = _dot(wsp_v[rr, :], r[0:S, FH + c * TN:FH + (c + 1) * TN])
        bb = bcol[rr, :]
        gg = gg + jnp.concatenate([bb] * (TN // 128), axis=1)
        ml[:, cs] = _pack((r[rr, cs].astype(f32) * gg).astype(bf16))

    def o_chunk(src, dst, dst_c, i, c):
        cs = slice(c * TN, (c + 1) * TN)
        rr = rows_of(i)
        o = _dot(_unpack(ml[...]), wout_v[:, cs])
        x = src[rr, XC + c * TN:XC + (c + 1) * TN].astype(f32) + o
        dst[rr, dst_c + c * TN:dst_c + (c + 1) * TN] = x.astype(bf16)

    nzh = FH // TN
    noc = D // TN
    parts_z = _spread(list(range(npc)), nzh)
    parts_o = _spread(list(range(npc)), noc)

    q_copy.wait()
    for ps in parts_z:
        a_layer_piece(r1, 0, 0, ps, 0)
    win_copy.wait()

    def p1_body(i, carry):
        iy = jnp.minimum(i + 1, NR - 1)
        xnl[...] = _pack(r1[rows_of(i), 0:D])
        for c in range(nzh):
            a_layer_piece(r1, i + 1, iy, parts_z[c], 0)
            z_chunk(r1, i, nzh + c)
        for c in range(nzh):
            norm_piece(r1, i, parts_z[c])
            z_chunk(r1, i, c)
        return carry

    jax.lax.fori_loop(0, NR, p1_body, 0)

    wsp_copy.wait()
    wout_copy.wait()

    for c in range(nzh):
        g_chunk(r1, 0, c)
    for c in range(noc):
        o_chunk(r1, r2, XC, 0, c)
    for ps in parts_z:
        a_layer_piece(r2, 0, 0, ps, FH)

    def p2_body(i, carry):
        xnl[...] = _pack(r2[rows_of(i - 1), FH:FH + D])
        for c in range(nzh):
            g_chunk(r1, i, c)
        for c in range(nzh):
            z_chunk(r2, i - 1, nzh + c)
        for c in range(noc):
            norm_piece(r2, i - 1, parts_o[c])
            o_chunk(r1, r2, XC, i, c)
        for c in range(nzh):
            a_layer_piece(r2, i, i, parts_z[c], FH)
            z_chunk(r2, i - 1, c)
        return carry

    jax.lax.fori_loop(1, NR, p2_body, 0)

    last = NR - 1
    xnl[...] = _pack(r2[rows_of(last), FH:FH + D])
    for c in range(nzh):
        z_chunk(r2, last, nzh + c)
    for c in range(nzh):
        norm_piece(r2, last, parts_z[c])
        z_chunk(r2, last, c)

    for c in range(nzh):
        g_chunk(r2, 0, c)

    def p3_body(i, carry):
        for c in range(noc):
            o_chunk(r2, y_v, 0, i - 1, c)
        out_copy(i - 1).start()
        for c in range(nzh):
            g_chunk(r2, i, c)
        return carry

    jax.lax.fori_loop(1, NR, p3_body, 0)
    for c in range(noc):
        o_chunk(r2, y_v, 0, NR - 1, c)
    out_copy(NR - 1).start()
    for i in range(NR):
        out_copy(i).wait()


@jax.jit
def pallas_interleave_layers__ssm_conv_h3__mixer_gmlp__prompt_kernel(
    A_q: jax.Array,
    A_k: jax.Array,
    A_v: jax.Array,
    A_shift_k: jax.Array,
    A_ssm_k: jax.Array,
    A_ssm_D: jax.Array,
    B_x: jax.Array,
    B_w_in: jax.Array,
    B_w_sp: jax.Array,
    B_b_sp: jax.Array,
    B_w_out: jax.Array,
):
    del B_x
    anyspec = pl.BlockSpec(memory_space=pl.ANY)
    vmem = pl.BlockSpec(memory_space=pltpu.VMEM)
    u32 = jnp.uint32
    return pl.pallas_call(
        _kernel,
        grid=(1,),
        in_specs=[anyspec, anyspec, anyspec, vmem, anyspec, vmem, anyspec, anyspec, vmem,
                  anyspec, vmem],
        out_specs=anyspec,
        out_shape=jax.ShapeDtypeStruct((1, S, D), bf16),
        scratch_shapes=[
            pltpu.VMEM((S, D), bf16),
            pltpu.VMEM((S, D), bf16),
            pltpu.VMEM((D, S), bf16),
            pltpu.VMEM((D, F), bf16),
            pltpu.VMEM((S, S), bf16),
            pltpu.VMEM((FH, D), bf16),
            pltpu.VMEM((S, D), bf16),
            pltpu.VMEM((S + TM, RW), bf16),
            pltpu.VMEM((S, RW), bf16),
            pltpu.VMEM((TM // 2, D), u32),
            pltpu.VMEM((TM // 2, FH), u32),
            pltpu.VMEM((7, NB + 1, P, 128), f32),
            pltpu.VMEM((7, NB + 1, P, 128), f32),
            pltpu.VMEM((S, 128), bf16),
            pltpu.VMEM((S, 128), bf16),
            pltpu.VMEM((S, 128), bf16),
            pltpu.VMEM((S + 8, 128), f32),
            pltpu.VMEM((7 * P // 2, 128), u32),
            pltpu.VMEM((S, 128), f32),
            pltpu.SemaphoreType.DMA((NG,)),
            pltpu.SemaphoreType.DMA((NG,)),
            pltpu.SemaphoreType.DMA((NG,)),
            pltpu.SemaphoreType.DMA((4,)),
            pltpu.SemaphoreType.DMA((NR,)),
        ],
        compiler_params=pltpu.CompilerParams(
            dimension_semantics=("arbitrary",),
            vmem_limit_bytes=120 * 1024 * 1024,
        ),
    )(A_q, A_k, A_v, A_shift_k.T, A_ssm_k, A_ssm_D, B_w_in, B_w_sp, B_b_sp, B_w_out,
      _dft_constants())
```

```python
import numpy as np
import jax
import jax.numpy as jnp
import jax.experimental.pallas as pl
import jax.experimental.pallas.tpu as pltpu

S = 2048
D = 1024
F = 3584
FH = F // 2
P = 128
NB = S // P
HB = NB // 2
HS = S // 2
NG = D // 128
TM = 256
NR = S // TM
TN = 256
PR = 16
XC = F
RW = F + D
NT = FH // 128
EPS = 1e-5

STOP = 0
H3PRE = 1
PREPIN = 0
KS = 2
TPS = 8
W0 = 0.5
LNP = 7
LND = 2
TN1 = 128
BM = 'q4'
ONLY = ''
XTOK = 1
PSP = 2
KQ = 4
WC = 1.0
LAG = 2
REL = 0
LLAG = 8
LREL = 0
LDN = 1
LNM = 0
HARD = 1
ALT = 1
NOLN = 0
KQ0 = 2
PSP0 = 1
RPT0 = 16
LAG0 = 2
TNC = 256
LNA = 7
H3P1 = 0
ORDER = "H0 lo0 H1 mi0 H2 lo1 C0 mi1 P0 U0 lo2 mi2 U1 lo3 C1 mi3 P1".split()
P1ORD = 'CUHPKB'
W1 = 2
DORD = 3
DYNB = 1
NOW = 0
MAN = 2
DEFN = 2
LNH = 4
U2 = 1
U1 = 1
OSP = 1
U3 = 2
TR2 = 0
TR1 = 0
TINY = 0
LATE = 1

BS = 76
OY = 48
OT = 75
OO = 58
OK_ = 66
PB = 2 * BS
OD = 2 * BS
YT = 4 * PB
TK = YT + 54
NTW = TK + NR
Z1 = 0
Z2 = Z1 + NT * NR
YV = Z2 + NT * (NR + 1)
NTZ = YV + NR * NG


def band(n):
    return n * BS


f32 = jnp.float32
bf16 = jnp.bfloat16
u32 = jnp.uint32


def _dft_constants():
    n = np.arange(P)
    k = np.concatenate([np.arange(0, P, 2), np.arange(1, P, 2)])
    ang = 2.0 * np.pi * np.outer(2 * k + 1, n) / (4 * P)
    fre, fim = np.cos(ang), -np.sin(ang)
    fu = np.concatenate([fre, fim], 0)
    fh = np.concatenate([fre, fim - fre, fre + fim], 0)
    g = np.concatenate([fre.T, fim.T], 0) / P
    return jnp.asarray(np.concatenate([fu, fh, g], 0), dtype=bf16)


def _ln(x):
    m = jnp.mean(x, axis=-1, keepdims=True)
    xc = x - m
    v = jnp.mean(xc * xc, axis=-1, keepdims=True)
    return xc * jax.lax.rsqrt(v + EPS)


def _gelu(z):
    c = 0.7978845608028654
    u = z * (c + (c * 0.044715) * (z * z))
    h = 0.5 * z
    return h + h * jnp.tanh(u)


def _dot(a, b):
    return jnp.dot(a, b, preferred_element_type=f32)


def _spread(work, n):
    return [work[(j * len(work)) // n:((j + 1) * len(work)) // n] for j in range(n)]


def _dot_nt(a, b):
    return jax.lax.dot_general(a, b, (((1,), (1,)), ((), ())), preferred_element_type=f32)


def _pack(x):
    return pltpu.bitcast(x, u32)


def _unpack(x):
    return pltpu.bitcast(x, bf16)


def _f(x):
    return pltpu.bitcast(x, f32)


def _kernel(q_hbm, k_hbm, v_hbm, shk_hbm, hk_hbm, dv_hbm, win_hbm, wsp_hbm, bsp_hbm,
            wout_hbm, dft_hbm, out_hbm,
            win_v, wsp_v, wout_v, y_v, r1, r2, xnl, ml,
            w, uhh, kv0, kv1, kv2, kvh, cbuf, kf_s, dft_p, bcol, par, zs,
            shk_ref, dv_ref, bsp_ref, dft_ref,
            sem_k, sem_v, sem_h, sem_w, sem_q, sem_o, sem_s):
    small = [pltpu.make_async_copy(a, b, sem_s.at[j]) for j, (a, b) in enumerate(
        [(shk_hbm, shk_ref), (dv_hbm, dv_ref), (bsp_hbm, bsp_ref), (dft_hbm, dft_ref)])]
    for c in (small if MAN == 1 else [small[0], small[3]]):
        c.start()
    def lanes(g, off=0):
        if isinstance(g, int):
            return slice(off + g * 128, off + (g + 1) * 128)
        return pl.ds(pl.multiple_of(off + g * 128, 128), 128)

    def grp_copies(g, h):
        cols, rows = lanes(g), slice(h * HS, (h + 1) * HS)
        s = h * NG + g
        hrows = slice(2 * D + h * HS, 2 * D + (h + 1) * HS)
        if TINY & 1:
            rows = slice(h * HS, h * HS + 128)
            hrows = slice(2 * D + h * HS, 2 * D + h * HS + 128)
        return (pltpu.make_async_copy(hk_hbm.at[cols, rows], r2.at[cols, hrows], sem_h.at[s]),
                pltpu.make_async_copy(k_hbm.at[0, rows, cols], r2.at[rows, cols], sem_k.at[s]),
                pltpu.make_async_copy(v_hbm.at[0, rows, cols], r2.at[rows, lanes(g, D)],
                                      sem_v.at[s]))

    def blk(i):
        if isinstance(i, int):
            return slice(i * TM, (i + 1) * TM)
        return pl.ds(pl.multiple_of(i * TM, TM), TM)

    def q_copy(i):
        return pltpu.make_async_copy(q_hbm.at[0, blk(i), :], r1.at[blk(i), XC:XC + D], sem_q.at[i])

    win_copy = [pltpu.make_async_copy(win_hbm.at[:, FH:F], win_v.at[:, FH:F], sem_w.at[0]),
                pltpu.make_async_copy(win_hbm.at[:, 0:FH], win_v.at[:, 0:FH], sem_w.at[1])]
    wsp_copy = pltpu.make_async_copy(wsp_hbm, wsp_v, sem_w.at[2])
    wout_copy = pltpu.make_async_copy(wout_hbm, wout_v, sem_w.at[3])

    if TINY & 2:
        win_copy = [pltpu.make_async_copy(win_hbm.at[0:16, FH:F], win_v.at[0:16, FH:F], sem_w.at[0]),
                    pltpu.make_async_copy(win_hbm.at[0:16, 0:FH], win_v.at[0:16, 0:FH], sem_w.at[1])]
    if TINY & 4:
        wsp_copy = pltpu.make_async_copy(wsp_hbm.at[0:16], wsp_v.at[0:16], sem_w.at[2])
        wout_copy = pltpu.make_async_copy(wout_hbm.at[0:16], wout_v.at[0:16], sem_w.at[3])

    def out_copy(i):
        return pltpu.make_async_copy(y_v.at[blk(i), :], out_hbm.at[0, blk(i), :], sem_o.at[i])

    def start(cs):
        for c in cs:
            c.start()

    def wait(cs):
        for c in cs:
            c.wait()

    lo = lambda g: list(grp_copies(g, 0))
    hi = lambda g: list(grp_copies(g, 1))
    if DORD == 0:
        sched = {-1: sum([lo(g) for g in range(NG)], []) + hi(0) + hi(1)
                 + [q_copy(0), q_copy(1), win_copy[0]] + hi(2) + [win_copy[1]] + hi(3)}
    elif DORD == 1:
        sched = {-1: lo(0) + lo(1), 0: lo(2) + lo(3) + lo(4), 1: lo(5) + lo(6) + lo(7),
                 2: hi(0) + hi(1) + [q_copy(0), q_copy(1), win_copy[0]],
                 4: hi(2) + [win_copy[1]] + hi(3)}
    elif DORD == 3:
        sched = {-1: lo(0), -0.5: lo(1), 0: lo(2) + lo(3) + lo(4), 1: lo(5) + lo(6) + lo(7),
                 2: hi(0) + hi(1) + [q_copy(0), q_copy(1), win_copy[0]],
                 4: hi(2) + [win_copy[1]] + hi(3)}
    elif DORD == 4:
        sched = {-1: lo(0), 0: lo(1) + lo(2), 1: lo(3) + lo(4) + lo(5), 2: lo(6) + lo(7) + hi(0) + hi(1),
                 3: [q_copy(0), q_copy(1), win_copy[0]],
                 5: hi(2) + [win_copy[1]] + hi(3)}
    elif DORD == 5:
        sched = {-1: lo(0), -0.5: lo(1), 0: lo(2) + lo(3), 1: lo(4) + lo(5) + [win_copy[0]], 3: lo(6) + lo(7),
                 4: hi(0) + hi(1) + [q_copy(0), q_copy(1)],
                 5: hi(2) + [win_copy[1]] + hi(3)}
    elif DORD == 2:
        sched = {-1: lo(0) + lo(1) + lo(2), 0: lo(3) + lo(4) + [win_copy[0]], 2: lo(5) + lo(6),
                 3: lo(7) + hi(0) + hi(1) + [q_copy(0), q_copy(1)],
                 5: hi(2) + [win_copy[1]] + hi(3)}
    start(sched[-1])
    if MAN == 2:
        start(small[1:3])

    kvs = [kv0, kv1, kv2]
    r1[S:S + TM, XC:XC + D] = jnp.zeros((TM, D), bf16)
    wait(small if MAN == 1 else [small[0], small[3]])
    start(sched.get(-0.5, []))
    for j in range(8):
        zs[j] = 0
    zs[8] = 3
    zs[9] = 3 * PB
    zs[10] = TR2
    zs[12] = NR - 1
    zs[11] = TR1
    dft_p[...] = _pack(dft_ref[...])
    for g in range(NG):
        tp = shk_ref[:, lanes(g)].astype(f32)
        for j in range(4):
            w[band(g) + OT, 8 * j:8 * j + 8, :] = _pack(jnp.broadcast_to(tp[j:j + 1], (8, 128)))

    def setup2():
        drow = dv_ref[...].astype(f32).reshape(1, D)
        for g in range(NG):
            par[g] = jnp.broadcast_to(drow[:, lanes(g)], (8, 128))
        eye = (jax.lax.broadcasted_iota(jnp.int32, (128, 128), 0)
               == jax.lax.broadcasted_iota(jnp.int32, (128, 128), 1))
        brow = bsp_ref[...].astype(f32).reshape(1, S)
        for t in range(S // 128):
            row = jnp.broadcast_to(brow[:, t * 128:(t + 1) * 128], (128, 128))
            col = jnp.sum(jnp.where(eye, row, 0.0), axis=1, keepdims=True)
            bcol[t * 128:(t + 1) * 128, :] = jnp.broadcast_to(col, (128, 128))

    if MAN == 1:
        setup2()

    hp = P // 2
    dep = {"rv": None, "out": [], "keep": None}

    def rel(x, on=None):
        if dep["rv"] is None or not (REL if on is None else on):
            return x
        return jnp.where(dep["keep"], x, dep["rv"])

    def done(x, lag=LAG):
        if dep["rv"] is not None:
            dep["out"].append((lag, x))

    def rel2(x):
        if dep["rv"] is None or not LREL:
            return x
        return jnp.concatenate(
            [jnp.concatenate([rel(x[r:r + 8, 0:128], 1), x[r:r + 8, 128:]], 1)
             for r in range(0, x.shape[0], 8)], 0)

    def done2(xp):
        for r in range(0, xp.shape[0], 8):
            for j in range(0, xp.shape[1] // 128, LDN):
                done(_f(xp[r:r + 8, j * 128:(j + 1) * 128]), LLAG)

    class Stage:
        def __init__(self, g, g0, h, base, base2=None):
            self.g, self.g0, self.h, self.base = g, g0, h, base
            self.base2 = base if base2 is None else base2

        def uh(self, h):
            if h == 0:
                return w, self.base + band(self.g0)
            return uhh, (self.g0 % 2) * 48

        def yb(self, arr, t, pers):
            if pers:
                return self.base + band(self.g0) + OY + arr * 9 + (t - 7)
            return self.base + YT + (self.g0 % 2) * 27 + arr * 9 + (t + 1)

        def kv(self, b):
            if self.h == 0:
                return kvs[self.g % 3], (slice(b * hp, (b + 1) * hp), slice(None))
            return kvh, (self.g, slice(b * hp, (b + 1) * hp), slice(None))

        def dft(self, lo, n):
            return _unpack(dft_p[lo // 2:(lo + n) // 2, :])

    def h_mm(sa, b, h3):
        t0 = (sa.h * HB + b) * P
        hkb = r2[lanes(sa.g), 2 * D + t0:2 * D + t0 + P]
        dft = sa.dft
        if h3:
            return jnp.concatenate(
                [_dot_nt(dft(2 * P, 192), hkb), _dot_nt(dft(2 * P + 192, 192), hkb)], 0)
        c, d = _dot_nt(dft(0, P), hkb), _dot_nt(dft(P, P), hkb)
        return jnp.concatenate([c, d - c, c + d], 0)

    def h_store(sa, b, hd, lo, n):
        ref, o = sa.uh(sa.h)
        ref[o + (3 + lo // P) * 8 + b, lo % P:lo % P + n, :] = _pack(hd[lo:lo + n])

    def kv_make(sa, b, nb):
        cols = lanes(sa.g)
        t0 = (sa.h * HB + b) * P
        n = nb * P
        taps = par[sa.g]
        if t0 == 0:
            kf_s[0:8, :] = jnp.zeros((8, 128), f32)
        elif b == 0:
            kf_s[0:8, :] = r2[t0 - 16:t0, cols].astype(f32)[8:16]
        l0 = b * P + 8
        kf_s[l0:l0 + n, :] = r2[t0:t0 + n, cols].astype(f32)
        ks = kf_s[l0:l0 + n, :] * taps[0:1]
        for j in range(1, 4):
            ks = ks + kf_s[l0 - j:l0 - j + n, :] * taps[j:j + 1]
        kv = _pack((ks * r2[t0:t0 + n, lanes(sa.g, D)].astype(f32)).astype(bf16))
        for j in range(nb):
            ref, idx = sa.kv(b + j)
            ref[idx] = kv[j * hp:(j + 1) * hp]

    def kv_fine(sa, b, q, nq):
        cols = lanes(sa.g)
        n = P // nq
        t0 = (sa.h * HB + b) * P + q * n
        l0 = b * P + q * n + 8
        if t0 == 0:
            kf_s[0:8, :] = jnp.zeros((8, 128), f32)
        elif l0 == 8:
            kf_s[0:8, :] = r2[t0 - 16:t0, cols].astype(f32)[8:16]
        kf_s[l0:l0 + n, :] = r2[t0:t0 + n, cols].astype(f32)
        tb = sa.base + band(sa.g0) + OT
        ks = None
        for j in range(4):
            tj = jnp.concatenate([rel(_f(w[tb, 8 * j:8 * j + 8, :]))] * (n // 8), 0)
            term = kf_s[l0 - j:l0 - j + n, :] * tj
            ks = term if ks is None else ks + term
        kv = _pack((ks * r2[t0:t0 + n, lanes(sa.g, D)].astype(f32)).astype(bf16))
        o = (b * P + q * n) // 2
        if sa.h:
            kvh[sa.g, o:o + n // 2, :] = kv
        else:
            kvs[sa.g % 3][o:o + n // 2, :] = kv
        for j in range(n // 16):
            done(_f(kv[8 * j:8 * j + 8]))

    def u_mm(sa, b):
        ref, idx = sa.kv(b)
        kvb = _unpack(ref[idx])
        return _dot(sa.dft(0, P), kvb), _dot(sa.dft(P, P), kvb)

    def u_store(sa, b, u, rr):
        ref, o = sa.uh(sa.h)
        for a in range(2):
            ref[o + a * 8 + b, rr, :] = _pack(u[a][rr])
        ref[o + 16 + b, rr, :] = _pack(u[0][rr] + u[1][rr])

    def c_prep(sb, sp, dup, bs=range(HB)):
        pers = sb.h == 1
        r = slice(sp * 16, sp * 16 + 16)
        pk = slice(sp * 8, sp * 8 + 8)
        pk2 = slice(hp + sp * 8, hp + sp * 8 + 8)

        def ld(t):
            s1, s3, s2 = (_f(w[sb.yb(a, t, pers), r, :]) for a in range(3))
            s1 = jnp.concatenate([rel(s1[0:8]), rel(s1[8:16])], 0)
            return s1 - s3, s1 + s2

        t0 = sb.h * HB + bs[0]
        prev = ld(t0 - 1) if t0 else None
        for b in bs:
            t = sb.h * HB + b
            cr, ci = ld(t)
            if prev is None:
                a, c = cr, ci
            elif sp < 4:
                a, c = cr - prev[1], ci + prev[0]
            else:
                a, c = cr + prev[1], ci - prev[0]
            prev = (cr, ci)
            a, c = _pack(a.astype(bf16)), _pack(c.astype(bf16))
            n = (sb.g0 % 2) * HB + b
            cbuf[n, pk, :] = a
            cbuf[n, pk2, :] = c
            done(_f(a))
            done(_f(c))

    def c_mm(sc, b, tok=None):
        dft = sc.dft
        n = (sc.g0 % 2) * HB + b
        a, c = _unpack(cbuf[n, 0:hp, :]), _unpack(cbuf[n, hp:P, :])
        yt = _dot(dft(5 * P, P), a) + _dot(dft(6 * P, P), c)
        if tok:
            yt = tok(yt)
        ref, idx = sc.kv(b)
        kv = _unpack(ref[idx]).astype(f32)
        return (yt + kv * par[sc.g][4:5]).astype(bf16)

    def c_store(sc, b, y):
        t0 = (sc.h * HB + b) * P
        y_v[t0:t0 + P, lanes(sc.g)] = y

    def b_terms(sb, sl, arr, terms, init):
        r = slice(sl * 8, sl * 8 + 8)
        ha, ua = [(0, 2), (2, 1), (1, 0)][arr]
        out, hs, us, seen = {}, {}, {}, set()
        for t, uh_, b, hh_, d in terms:
            if t not in out and init(t):
                out[t] = _f(w[sb.yb(arr, t, True), r, :])
            if (hh_, d) not in hs:
                hr, ho = sb.uh(hh_)
                hs[hh_, d] = _f(hr[ho + (3 + ha) * 8 + d, r, :])
                if REL == 2:
                    hs[hh_, d] = rel(hs[hh_, d])
            if (uh_, b) not in us:
                ur, uo = sb.uh(uh_)
                us[uh_, b] = _f(ur[uo + ua * 8 + b, r, :])
            term = hs[hh_, d] * us[uh_, b]
            if t not in seen and REL == 1:
                term = rel(term)
            seen.add(t)
            out[t] = out[t] + term if t in out else term
        for t, val in out.items():
            done(val)
            if t <= 7:
                w[sb.yb(arr, t, False), r, :] = _pack(val)
            if t >= 7:
                w[sb.yb(arr, t, True), r, :] = _pack(val)

    def mk_terms(ts, sets, bs=range(8)):
        return [(t, uh_, b, hh_, t - 8 * uh_ - 8 * hh_ - b) for uh_, hh_ in sets for t in ts
                for b in bs if 0 <= t - 8 * uh_ - 8 * hh_ - b <= 7]

    def b_slice(sb, sl, kind, split=False):
        ab = [(1, 0), (0, 1)]
        if kind == "lo":
            groups = [(mk_terms(range(0, 8), [(0, 0)]), lambda t: False)]
        elif kind == "mi":
            groups = [(mk_terms(range(8, 15), [(0, 0)]), lambda t: False)]
        elif not split or BM == "pass":
            groups = [(mk_terms(range(8, 16), ab), lambda t: t < 15)]
        elif BM == "q4":
            groups = [(mk_terms(range(8, 12), ab), lambda t: True),
                      (mk_terms(range(12, 16), ab[:1], range(0, 4)), lambda t: t < 15),
                      (mk_terms(range(12, 16), ab[1:], range(0, 4)), lambda t: True),
                      (mk_terms(range(12, 16), ab, range(4, 8)), lambda t: True)]
        else:
            groups = [(mk_terms(range(8, 16), ab[:1]), lambda t: t < 15),
                      (mk_terms(range(8, 16), ab[1:]), lambda t: True)]
        fs = [lambda arr=arr, g=g: b_terms(sb, sl, arr, *g) for g in groups for arr in range(3)]
        if split:
            return fs
        for f in fs:
            f()

    def static_stage(s, zi):
        if s < 0 or s >= 2 * NG:
            return None
        if PREPIN == 0:
            return Stage(s % NG, s % NG, s // NG, 0)
        return Stage(s % NG, s % NG, s // NG, zab[min(zi, 1)], zab[0])

    def conv_pieces(sa, sb, sc, frac=1.0, h3=0, kq=KQ, psp=PSP):
        def hu(b, tok):
            hd = h_mm(sa, b, h3)
            u = u_mm(sa, b)
            u = (tok(u[0]), u[1])
            for a in range(3):
                h_store(sa, b, hd, a * P, P)
            u_store(sa, b, u, slice(0, P))

        def cc(b, tok):
            ys = [c_mm(sc, b + j, tok if j == 0 else None) for j in range(2)]
            for j in range(2):
                c_store(sc, b + j, ys[j])

        mx, out = [], []
        d = 1.0 / (HB + 1.0)
        for b in range(HB):
            if sa:
                kvp = [lambda b=b, q=q: kv_fine(sa, b, q, kq) for q in range(kq)]
                mx.append(((b + 1.2) * d, lambda tok, b=b: hu(b, tok), kvp))
                out += [((b + q / kq) * d, 200 / kq, f) for q, f in enumerate(kvp)]
            if sc and b % 2 == 0:
                mx.append((b / HB * frac, lambda tok, b=b: cc(b, tok), []))
        if sb:
            for sl in range(2 * HB):
                fs = b_slice(sb, sl, "hi", True) if sb.h else (
                    b_slice(sb, sl, "lo", True) + b_slice(sb, sl, "mi", True))
                fs = [(432.0 / len(fs), f) for f in fs]
                if sl % 2:
                    fs = fs + [(130 / psp, lambda sl=sl, bs=bs: c_prep(sb, sl // 2, True, bs))
                               for bs in _spread(list(range(HB)), psp)]
                for j, (c_, f) in enumerate(fs):
                    out.append(((sl + j / len(fs)) / (2.0 * HB), c_, f))
        return sorted(mx, key=lambda x: x[0]), sorted(out, key=lambda x: x[0])

    def scheduler(wts, pieces, rpt, lag):
        cum = np.cumsum(wts) / np.sum(wts)
        slots = [[] for _ in wts]
        tot, run = sum(c_ for _, c_, _ in pieces), 0.0
        for _, c_, f in pieces:
            slots[min(int(np.searchsorted(cum, run / tot, side="right")), len(wts) - 1)].append(f)
            run += c_
        pend, cnt, ran = [], [0], []
        keep = jnp.full((8, 128), zs[5], jnp.int32) == 0

        def call(f):
            if not any(f is g for g in ran):
                ran.append(f)
                f()

        def need(fs):
            for f in fs:
                call(f)

        def tok(val):
            if not pieces:
                return val
            tiles = [val[r0:r0 + 8] for r0 in range(0, val.shape[0], 8)]
            for r0 in range(0, val.shape[0], rpt):
                due = [v for n, v in pend if n <= cnt[0]]
                pend[:] = [e for e in pend if e[0] > cnt[0]]
                for j, v in enumerate(due):
                    q = r0 // 8 + j % (rpt // 8)
                    tiles[q] = jnp.where(keep, tiles[q], v)
                dep["rv"], dep["out"], dep["keep"] = val[r0:r0 + 8], [], keep
                for f in slots[cnt[0]]:
                    call(f)
                pend.extend((cnt[0] + lag, v) for _, v in dep["out"])
                dep["rv"] = None
                cnt[0] += 1
            return jnp.concatenate(tiles, 0)

        return tok, need

    for s in range(NG + 2):
        if not (NOW & 1 and s > 0 or NOW & 4):
            wait(grp_copies(s % NG, s // NG))
        start(sched.get(s, []))
        if MAN == 2 and s == 0:
            wait(small[1:3])
            setup2()
        if ONLY:
            continue
        mx, pieces = conv_pieces(static_stage(s, 0), static_stage(s - 1, 1),
                                 static_stage(s - 2, 2), h3=H3PRE, kq=KQ0, psp=PSP0)
        tok, need = scheduler([1.0] * (len(mx) * P // RPT0), pieces, RPT0, LAG0)
        for _, f, pre in mx:
            need(pre)
            f(tok)

    npc = TM // PR

    def rows_of(i, r0=0, nr=TM):
        return pl.ds(pl.multiple_of(i * TM + r0, PR), nr)

    def a_layer_piece(r, i, iy, ps, stage_c):
        if not ps:
            return
        rr = rows_of(i, ps[0] * PR, len(ps) * PR)
        ry = rows_of(iy, ps[0] * PR, len(ps) * PR)
        x = r[rr, XC:XC + D].astype(f32)
        x = x + _ln(x) * y_v[ry, :].astype(f32)
        r[rr, XC:XC + D] = x.astype(bf16)
        r[rr, stage_c:stage_c + D] = _ln(x).astype(bf16)

    def norm_piece(r, i, ps):
        if not ps:
            return
        rr = rows_of(i, ps[0] * PR, len(ps) * PR)
        r[rr, FH:F] = _ln(r[rr, FH:F].astype(f32)).astype(bf16)

    nzh = FH // TN
    noc = D // TN

    def z_chunk(r, i, c, tn=TN, tok=lambda v: v, ks=1):
        cs = slice(c * tn, (c + 1) * tn)
        kk = D // ks
        acc = None
        for k in range(ks):
            part = _dot(_unpack(xnl[:, k * kk:(k + 1) * kk]), win_v[k * kk:(k + 1) * kk, cs])
            if tn > 128 and ks > 1:
                part = jnp.concatenate([tok(part[:, 0:128]), part[:, 128:]], 1)
            else:
                part = tok(part)
            acc = part if acc is None else acc + part
        r[rows_of(i), cs] = _gelu(acc).astype(bf16)

    def g_chunk(r, i, c):
        cs = slice(c * TN, (c + 1) * TN)
        rr = rows_of(i)
        gg = _dot(wsp_v[rr, :], r[0:S, FH + c * TN:FH + (c + 1) * TN])
        bb = bcol[rr, :]
        gg = gg + jnp.concatenate([bb] * (TN // 128), axis=1)
        ml[:, cs] = _pack((r[rr, cs].astype(f32) * gg).astype(bf16))

    def o_chunk(src, dst, dst_c, i, c):
        cs = slice(c * TN, (c + 1) * TN)
        rr = rows_of(i)
        o = _dot(_unpack(ml[...]), wout_v[:, cs])
        x = src[rr, XC + c * TN:XC + (c + 1) * TN].astype(f32) + o
        dst[rr, dst_c + c * TN:dst_c + (c + 1) * TN] = x.astype(bf16)

    parts_z = _spread(list(range(npc)), nzh)
    parts_o = _spread(list(range(npc)), noc)

    def finish(pending):
        wait(pending)
        out_copy(NR - 1).start()
        out_copy(NR - 1).wait()

    late = sum([hi(g) for g in range(4, NG)], []) + [q_copy(i) for i in range(2, NR)]
    if not LATE:
        start(late)
    if not NOW & 2:
        q_copy(0).wait()
    for ps in parts_z:
        a_layer_piece(r1, 0, 0, ps, 0)
    if not NOW & 2:
        wait(win_copy if W1 == 0 else win_copy[:1])
    if STOP == 1:
        finish([c for g in range(2, NG) for c in grp_copies(g, 1)] + [q_copy(i) for i in range(1, NR)])
        return
    if not LATE:
        start([wsp_copy, wout_copy])

    def ln_pieces(fn, lo=0.0, hi=1.0, n=LNP, sub=None):
        d = (hi - lo) / n
        return [(lo + j * d, lambda ps=ps: fn(ps))
                for j, ps in enumerate(_spread(sub or list(range(npc)), n))]

    def p1_half(i, hh, lnp, conv=((), ())):
        mx, pieces = conv
        if NOLN & (1 << hh) and pieces:
            lnp = []
        tn = TN1 if pieces else TNC
        nz1 = FH // tn
        ks = 2 * tn // 128
        rpt = TM // TPS
        grp = [[e for e in mx if min(int(e[0] * nz1 + 1e-6), nz1 - 1) == c] for c in range(nz1)]
        wts = []
        for c in range(nz1):
            wts += [WC] * (len(grp[c]) * P // rpt) + [1.0] * (TPS * (ks - 1)) + [W0] * TPS
        tok, need = scheduler(wts, pieces, rpt, LAG)
        for c in range(nz1):
            for p_, f in lnp:
                if min(int(p_ * nz1 + 1e-6), nz1 - 1) == c:
                    f()
            for _, f, pre in grp[c]:
                need(pre)
                f(tok)
            z_chunk(r1, i, c + (nz1 if hh == 0 else 0), tn, tok, ks if pieces else 1)

    def p1a_body(i, carry):
        if not NOW & 2:
            q_copy(i + 1).wait()
            wait(grp_copies(2 * i + 2, 1))
        if W1 < 2:
            wait(grp_copies(2 * i + 3, 1))
        base = i * PB

        def st(g0):
            return Stage(2 * i + g0, g0, 1, base)

        xnl[...] = _pack(r1[rows_of(i), 0:D])
        al = lambda ps: a_layer_piece(r1, i + 1, i + 1, ps, 0)
        h0, h1 = list(range(npc // 2)), list(range(npc // 2, npc))
        p1_half(i, 0, ln_pieces(al, n=LNH, sub=h0) if DEFN == 2 else ln_pieces(al, n=LNA),
                conv_pieces(st(2), st(1), st(0)))
        if W1 >= 2 and not NOW & 2:
            wait(grp_copies(2 * i + 3, 1))
        if W1 == 2:
            @pl.when(i == 0)
            def _():
                if not NOW & 2:
                    win_copy[1].wait()
                if LATE:
                    start(late)
        p1_half(i, 1, [ln_pieces(lambda ps: norm_piece(r1, i, ps), n=LNA), [],
                       ln_pieces(al, n=LNH, sub=h1)][DEFN],
                conv_pieces(st(3), st(2), st(1)))
        return carry

    if ONLY != 'p1c':
        jax.lax.fori_loop(0, 3, p1a_body, 0)
    else:
        wait([q_copy(i) for i in range(1, 4)] + [c for g in range(2, NG) for c in grp_copies(g, 1)])

    if W1 in (1, 3):
        win_copy[1].wait()
    if LATE:
        start([wsp_copy, wout_copy])
    if NOW & 2:
        wait(win_copy + [q_copy(i) for i in range(4)] + sum([hi(g) for g in range(2, NG)], []))
    if NOW & 5:
        wait(sum([list(grp_copies(s % NG, s // NG)) for s in range(0 if NOW & 4 else 1, NG + 2)], []))
    wait([q_copy(i) for i in range(4, NR)])
    if ONLY == 'p1a':
        finish([wsp_copy, wout_copy])
        return
    i3 = zs[8]
    xnl[...] = _pack(r1[rows_of(i3), 0:D])
    if DYNB:
        b3 = zs[9]
        s14, s15 = Stage(2 * i3, 0, 1, b3), Stage(2 * i3 + 1, 1, 1, b3)
    else:
        s14, s15 = static_stage(14, 0), static_stage(15, 0)
    p1_half(i3, 0, [], conv_pieces(None, s15, s14))
    p1_half(i3, 1, ([] if DEFN else ln_pieces(lambda ps: norm_piece(r1, i3, ps), 0.0, 0.5, 4))
            + ln_pieces(lambda ps: a_layer_piece(r1, i3 + 1, i3 + 1, ps, 0), 0.45, 1.0, 4),
            conv_pieces(None, None, s15, 0.4))

    def p1c_body(i, carry):
        iy = jnp.minimum(i + 1, NR - 1)
        xnl[...] = _pack(r1[rows_of(i), 0:D])
        p1_half(i, 0, ln_pieces(lambda ps: a_layer_piece(r1, i + 1, iy, ps, 0)))
        p1_half(i, 1, ln_pieces(lambda ps: norm_piece(r1, i, ps))
                + (ln_pieces(lambda ps: norm_piece(r1, i - 4, ps)) if DEFN else []))
        return carry

    if U1 == 1:
        jax.lax.fori_loop(4, zs[11] if TR1 else NR, p1c_body, 0)
    else:
        jax.lax.fori_loop(2, 4, lambda j, cr: p1c_body(2 * j + 1, p1c_body(2 * j, cr)), 0)

    wsp_copy.wait()
    wout_copy.wait()
    if STOP == 2:
        finish([])
        return

    for c in range(nzh):
        g_chunk(r1, 0, c)
    for c in range(noc):
        o_chunk(r1, r2, XC, 0, c)
    for ps in parts_z:
        a_layer_piece(r2, 0, 0, ps, FH)

    def p2_body(i, carry):
        xnl[...] = _pack(r2[rows_of(i - 1), FH:FH + D])
        for c in range(nzh):
            g_chunk(r1, i, c)
        for c in range(nzh):
            z_chunk(r2, i - 1, nzh + c)
        for c in range(noc):
            norm_piece(r2, i - 1, parts_o[c])
            o_chunk(r1, r2, XC, i, c)
        for c in range(nzh):
            a_layer_piece(r2, i, i, parts_z[c], FH)
            z_chunk(r2, i - 1, c)
        return carry

    if U2 == 1:
        jax.lax.fori_loop(1, zs[10] if TR2 else NR, p2_body, 0)
    else:
        jax.lax.fori_loop(0, 3, lambda j, cr: p2_body(2 * j + 2, p2_body(2 * j + 1, cr)), 0)
        p2_body(zs[12], 0)

    last = NR - 1
    xnl[...] = _pack(r2[rows_of(last), FH:FH + D])
    for c in range(nzh):
        z_chunk(r2, last, nzh + c)
    for c in range(nzh):
        norm_piece(r2, last, parts_z[c])
        z_chunk(r2, last, c)

    for c in range(nzh):
        g_chunk(r2, 0, c)

    def p3_body(i, carry):
        for c in range(noc):
            o_chunk(r2, y_v, 0, i - 1, c)
        out_copy(i - 1).start()
        for c in range(nzh):
            g_chunk(r2, i, c)
        return carry

    if U3 == 1:
        jax.lax.fori_loop(1, NR, p3_body, 0)
    elif U3 == 2:
        jax.lax.fori_loop(0, 3, lambda j, cr: p3_body(2 * j + 2, p3_body(2 * j + 1, cr)), 0)
        p3_body(NR - 1, 0)
    else:
        for i in range(1, NR):
            p3_body(i, 0)
    def out_last(c):
        cs = slice(c * TN, (c + 1) * TN)
        return pltpu.make_async_copy(y_v.at[blk(last), cs], out_hbm.at[0, blk(last), cs],
                                     sem_o.at[NR + c])

    for c in range(noc):
        o_chunk(r2, y_v, 0, NR - 1, c)
        if OSP:
            out_last(c).start()
    if not OSP:
        out_copy(NR - 1).start()
    for i in range(NR - OSP):
        out_copy(i).wait()
    if OSP:
        wait([out_last(c) for c in range(noc)])


@jax.jit
def pallas_interleave_layers__ssm_conv_h3__mixer_gmlp__prompt_kernel(
    A_q, A_k, A_v, A_shift_k, A_ssm_k, A_ssm_D, B_x, B_w_in, B_w_sp, B_b_sp, B_w_out,
):
    del B_x
    anyspec = pl.BlockSpec(memory_space=pl.ANY)
    vmem = pl.BlockSpec(memory_space=pltpu.VMEM)
    return pl.pallas_call(
        _kernel,
        grid=(1,),
        in_specs=[anyspec] * 11,
        out_specs=anyspec,
        out_shape=jax.ShapeDtypeStruct((1, S, D), bf16),
        scratch_shapes=[
            pltpu.VMEM((D, F), bf16),
            pltpu.VMEM((S, S), bf16),
            pltpu.VMEM((FH, D), bf16),
            pltpu.VMEM((S, D), bf16),
            pltpu.VMEM((S + TM, RW), bf16),
            pltpu.VMEM((S, RW), bf16),
            pltpu.VMEM((TM // 2, D), u32),
            pltpu.VMEM((TM // 2, FH), u32),
            pltpu.VMEM((NTW, P, 128), u32),
            pltpu.VMEM((96, P, 128), u32),
            pltpu.VMEM((HS // 2, 128), u32),
            pltpu.VMEM((HS // 2, 128), u32),
            pltpu.VMEM((HS // 2, 128), u32),
            pltpu.VMEM((NG, HS // 2, 128), u32),
            pltpu.VMEM((2 * HB, P, 128), u32),
            pltpu.VMEM((HS + 8, 128), f32),
            pltpu.VMEM((7 * P // 2, 128), u32),
            pltpu.VMEM((S, 128), f32),
            pltpu.VMEM((NG, 8, 128), f32),
            pltpu.SMEM((16,), jnp.int32),
            pltpu.VMEM((4, D), bf16),
            pltpu.VMEM((D,), bf16),
            pltpu.VMEM((S,), bf16),
            pltpu.VMEM((7 * P, 128), bf16),
            pltpu.SemaphoreType.DMA((2 * NG,)),
            pltpu.SemaphoreType.DMA((2 * NG,)),
            pltpu.SemaphoreType.DMA((2 * NG,)),
            pltpu.SemaphoreType.DMA((5,)),
            pltpu.SemaphoreType.DMA((NR,)),
            pltpu.SemaphoreType.DMA((NR + 4,)),
            pltpu.SemaphoreType.DMA((4,)),
        ],
        compiler_params=pltpu.CompilerParams(
            dimension_semantics=("arbitrary",),
            vmem_limit_bytes=124 * 1024 * 1024,
        ),
    )(A_q, A_k, A_v, A_shift_k.T, A_ssm_k, A_ssm_D, B_w_in, B_w_sp, B_b_sp, B_w_out,
      _dft_constants())
```

```python
import numpy as np
import jax
import jax.numpy as jnp
import jax.experimental.pallas as pl
import jax.experimental.pallas.tpu as pltpu

S = 2048
D = 1024
F = 3584
FH = F // 2
P = 128
NB = S // P
HB = NB // 2
HS = S // 2
NG = D // 128
TM = 256
NR = S // TM
TN = 256
PR = 16
XC = F
RW = F + D
NT = FH // 128
EPS = 1e-5

STOP = 0
H3PRE = 0
MIG = 1
PREPIN = 0
KS = 2
TPS = 8
W0 = 0.8
LNP = 7
LND = 2
TN1 = 128
BM = 'q4'
ONLY = ''
XTOK = 1
PSP = 2
KQ = 4
WC = 1.0
LAG = 2
REL = 0
LLAG = 8
LREL = 0
LDN = 1
LNM = 0
HARD = 1
ALT = 1
NOLN = 0
KQ0 = 2
PSP0 = 1
RPT0 = 16
LAG0 = 2
TNC = 256
LNA = 7
H3P1 = 0
ORDER = "H0 lo0 H1 mi0 H2 lo1 C0 mi1 P0 U0 lo2 mi2 U1 lo3 C1 mi3 P1".split()
P1ORD = 'CUHPKB'
W1 = 2
DORD = 3
DYNB = 1
NOW = 0
MAN = 2
SPL0 = 0
BPRE = 0.15
MI = 2
WQ = 2
PAIR = 0
WB0 = '0 7 14'.split()
WB1 = '0 7 14'.split()
WST = '2 5 7 9'.split()
DW2 = 5
DW3 = 7
DW4 = 9
WQC = 7
CH = 600
CL = 250
LN1 = 0
PADW = 8
PS1 = 0
PS2 = 128
PS5 = 0
PS6 = 0
PS3 = 0
PS4 = 0
EPI = 0
KG = 4
PG = 2
ROT = 0
TRA = 0
NA2 = 2
TKF = 0
DEFN = 2
LNH = 4
U2 = 1
U1 = 1
OSP = 1
U3 = 2
TR2 = 0
TR1 = 0
TINY = 0
LATE = 1

BS = 76
OY = 48
OT = 75
OO = 58
OK_ = 66
PB = 2 * BS
OD = 2 * BS
YT = 4 * PB
TK = YT + 54
NTW = TK
Z1 = 0
Z2 = Z1 + NT * NR
YV = Z2 + NT * (NR + 1)
NTZ = YV + NR * NG


def band(n):
    return n * BS


f32 = jnp.float32
bf16 = jnp.bfloat16
u32 = jnp.uint32


def _dft_constants():
    n = np.arange(P)
    k = np.concatenate([np.arange(0, P, 2), np.arange(1, P, 2)])
    ang = 2.0 * np.pi * np.outer(2 * k + 1, n) / (4 * P)
    fre, fim = np.cos(ang), -np.sin(ang)
    fu = np.concatenate([fre, fim], 0)
    fh = np.concatenate([fre, fim - fre, fre + fim], 0)
    g = np.concatenate([fre.T, fim.T], 0) / P
    return jnp.asarray(np.concatenate([fu, fh, g], 0), dtype=bf16)


def _ln(x):
    m = jnp.mean(x, axis=-1, keepdims=True)
    if LN1:
        v = jnp.maximum(jnp.mean(x * x, axis=-1, keepdims=True) - m * m, 0.0)
        return (x - m) * jax.lax.rsqrt(v + EPS)
    xc = x - m
    v = jnp.mean(xc * xc, axis=-1, keepdims=True)
    return xc * jax.lax.rsqrt(v + EPS)


def _gelu(z):
    c = 0.7978845608028654
    u = z * (c + (c * 0.044715) * (z * z))
    h = 0.5 * z
    return h + h * jnp.tanh(u)


def _dot(a, b):
    return jnp.dot(a, b, preferred_element_type=f32)


def _spread(work, n):
    return [work[(j * len(work)) // n:((j + 1) * len(work)) // n] for j in range(n)]


def _dot_nt(a, b):
    return jax.lax.dot_general(a, b, (((1,), (1,)), ((), ())), preferred_element_type=f32)


def _pack(x):
    return pltpu.bitcast(x, u32)


def _unpack(x):
    return pltpu.bitcast(x, bf16)


def _f(x):
    return pltpu.bitcast(x, f32)


def _kernel(q_hbm, k_hbm, v_hbm, shk_hbm, hk_hbm, dv_hbm, win_hbm, wsp_hbm, bsp_hbm,
            wout_hbm, dft_hbm, out_hbm,
            win_v, wsp_v, wout_v, y_v, r1, r2, xnl, ml,
            w, uhh, kv0, kv1, kv2, kvh, cbuf, kf_s, dft_p, bcol, par, zs,
            shk_ref, dv_ref, bsp_ref, dft_ref,
            sem_k, sem_v, sem_h, sem_w, sem_q, sem_o, sem_s):
    small = [pltpu.make_async_copy(a, b, sem_s.at[j]) for j, (a, b) in enumerate(
        [(shk_hbm, shk_ref), (dv_hbm, dv_ref), (bsp_hbm, bsp_ref), (dft_hbm, dft_ref)])]
    for c in (small if MAN == 1 else [small[0], small[3]]):
        c.start()
    def lanes(g, off=0):
        if isinstance(g, int):
            return slice(off + g * 128, off + (g + 1) * 128)
        return pl.ds(pl.multiple_of(off + g * 128, 128), 128)

    def grp_copies(g, h):
        cols, rows = lanes(g), slice(h * HS, (h + 1) * HS)
        s = h * NG + g
        hrows = slice(2 * D + h * HS, 2 * D + (h + 1) * HS)
        if TINY & 1:
            rows = slice(h * HS, h * HS + 128)
            hrows = slice(2 * D + h * HS, 2 * D + h * HS + 128)
        if PAIR and isinstance(s, int) and 2 <= s < NG + 2:
            hc = pltpu.make_async_copy(hk_hbm.at[cols, rows], r2.at[cols, hrows], sem_h.at[s])
            if s % 2:
                return (hc,)
            c2 = slice(g * 128, (g + 2) * 128)
            return (hc, pltpu.make_async_copy(k_hbm.at[0, rows, c2], r2.at[rows, c2], sem_k.at[s]),
                    pltpu.make_async_copy(v_hbm.at[0, rows, c2],
                                          r2.at[rows, D + g * 128:D + (g + 2) * 128], sem_v.at[s]))
        return (pltpu.make_async_copy(hk_hbm.at[cols, rows], r2.at[cols, hrows], sem_h.at[s]),
                pltpu.make_async_copy(k_hbm.at[0, rows, cols], r2.at[rows, cols], sem_k.at[s]),
                pltpu.make_async_copy(v_hbm.at[0, rows, cols], r2.at[rows, lanes(g, D)],
                                      sem_v.at[s]))

    def lo0(part):
        r = slice(0, SPL0 * P) if part == 0 else slice(SPL0 * P, HS)
        hr = slice(2 * D + r.start, 2 * D + r.stop)
        sm = [sem_h.at[0], sem_k.at[0], sem_v.at[0]] if part else [sem_s.at[4 + j] for j in range(3)]
        return [pltpu.make_async_copy(hk_hbm.at[0:128, r], r2.at[0:128, hr], sm[0]),
                pltpu.make_async_copy(k_hbm.at[0, r, 0:128], r2.at[r, 0:128], sm[1]),
                pltpu.make_async_copy(v_hbm.at[0, r, 0:128], r2.at[r, D:D + 128], sm[2])]

    def blk(i):
        if isinstance(i, int):
            return slice(i * TM, (i + 1) * TM)
        return pl.ds(pl.multiple_of(i * TM, TM), TM)

    def q_copy(i):
        return pltpu.make_async_copy(q_hbm.at[0, blk(i), :], r1.at[blk(i), XC:XC + D], sem_q.at[i])

    win_copy = [pltpu.make_async_copy(win_hbm.at[:, FH:F], win_v.at[:, FH:F], sem_w.at[0]),
                pltpu.make_async_copy(win_hbm.at[:, 0:FH], win_v.at[:, 0:FH], sem_w.at[1])]
    wb = [[int(x) for x in WB0], [int(x) for x in WB1]]
    wpc = {}
    for hh_ in range(2):
        for a_, b_ in zip(wb[hh_][:-1], wb[hh_][1:]):
            cs_ = slice((1 - hh_) * FH + a_ * 128, (1 - hh_) * FH + b_ * 128)
            wpc[hh_, a_] = pltpu.make_async_copy(win_hbm.at[:, cs_], win_v.at[:, cs_],
                                                 sem_w.at[4 + len(wpc)])
    win_copy = [wpc[0, 0], wpc[1, 0]]
    wsp_copy = pltpu.make_async_copy(wsp_hbm, wsp_v.at[:, 0:S], sem_w.at[2])
    wout_copy = pltpu.make_async_copy(wout_hbm, wout_v.at[:, 0:D], sem_w.at[3])

    if TINY & 2:
        win_copy = [pltpu.make_async_copy(win_hbm.at[0:16, FH:F], win_v.at[0:16, FH:F], sem_w.at[0]),
                    pltpu.make_async_copy(win_hbm.at[0:16, 0:FH], win_v.at[0:16, 0:FH], sem_w.at[1])]
    if TINY & 4:
        wsp_copy = pltpu.make_async_copy(wsp_hbm.at[0:16], wsp_v.at[0:16], sem_w.at[2])
        wout_copy = pltpu.make_async_copy(wout_hbm.at[0:16], wout_v.at[0:16], sem_w.at[3])

    def out_copy(i):
        return pltpu.make_async_copy(y_v.at[blk(i), 0:D], out_hbm.at[0, blk(i), :], sem_o.at[i])

    def start(cs):
        for c in cs:
            c.start()

    def wait(cs):
        for c in cs:
            c.wait()

    lo = lambda g: list(grp_copies(g, 0))
    hi = lambda g: list(grp_copies(g, 1))
    if DORD == 0:
        sched = {-1: sum([lo(g) for g in range(NG)], []) + hi(0) + hi(1)
                 + [q_copy(0), q_copy(1), win_copy[0]] + hi(2) + [win_copy[1]] + hi(3)}
    elif DORD == 1:
        sched = {-1: lo(0) + lo(1), 0: lo(2) + lo(3) + lo(4), 1: lo(5) + lo(6) + lo(7),
                 2: hi(0) + hi(1) + [q_copy(0), q_copy(1), win_copy[0]],
                 4: hi(2) + [win_copy[1]] + hi(3)}
    elif DORD == 3:
        sched = {-1: lo(0), -0.5: lo(1), 0: lo(2) + lo(3) + lo(4), 1: lo(5) + lo(6) + lo(7),
                 2: hi(0) + hi(1) + [q_copy(0), q_copy(1), win_copy[0]],
                 4: hi(2) + [win_copy[1]] + hi(3)}
    elif DORD == 4:
        sched = {-1: lo(0), 0: lo(1) + lo(2), 1: lo(3) + lo(4) + lo(5), 2: lo(6) + lo(7) + hi(0) + hi(1),
                 3: [q_copy(0), q_copy(1), win_copy[0]],
                 5: hi(2) + [win_copy[1]] + hi(3)}
    elif DORD == 5:
        sched = {-1: lo(0), -0.5: lo(1), 0: lo(2) + lo(3), 1: lo(4) + lo(5) + [win_copy[0]], 3: lo(6) + lo(7),
                 4: hi(0) + hi(1) + [q_copy(0), q_copy(1)],
                 5: hi(2) + [win_copy[1]] + hi(3)}
    elif DORD == 6:
        sched = {-1: lo(0), -0.5: lo(1), 0: lo(2), 1: lo(3) + lo(4) + lo(5),
                 2: lo(6) + lo(7) + hi(0) + hi(1) + [q_copy(0), q_copy(1), win_copy[0]],
                 4: hi(2) + [win_copy[1]] + hi(3)}
    elif DORD == 2:
        sched = {-1: lo(0) + lo(1) + lo(2), 0: lo(3) + lo(4) + [win_copy[0]], 2: lo(5) + lo(6),
                 3: lo(7) + hi(0) + hi(1) + [q_copy(0), q_copy(1)],
                 5: hi(2) + [win_copy[1]] + hi(3)}
    if WQ:
        sched = {-1: lo(0), -0.5: lo(1), 0: lo(2) + lo(3) + lo(4), 1: lo(5) + lo(6) + lo(7),
                 2: hi(0) + hi(1) + [q_copy(0)]}
        assert len(WST) == len(wpc)
        for st_, (key_, c_) in zip(WST, wpc.items()):
            ex = [q_copy(1)] + hi(2) if key_ == (0, 0) else []
            pre_ = hi(3) if key_ == (1, 0) else []
            sched[int(st_)] = sched.get(int(st_), []) + pre_ + [c_] + ex
    if SPL0:
        sched[-1] = lo0(0) + lo0(1)
    start(sched[-1])
    if MAN == 2:
        start(small[1:3])

    kvs = [kv0, kv1, kv2]
    r1[S:S + TM, XC:XC + D] = jnp.zeros((TM, D), bf16)
    wait(small if MAN == 1 else [small[0], small[3]])
    start(sched.get(-0.5, []))
    for j in range(8):
        zs[j] = 0
    zs[8] = 3
    zs[9] = 3 * PB
    zs[10] = TR2
    zs[12] = NR - 1
    zs[13] = 0
    zs[14] = TRA
    zs[11] = TR1
    dft_p[...] = _pack(dft_ref[...])
    for g in range(NG):
        tp = shk_ref[:, lanes(g)].astype(f32)
        for j in range(4):
            w[band(g) + OT, 8 * j:8 * j + 8, :] = _pack(jnp.broadcast_to(tp[j:j + 1], (8, 128)))

    def setup2():
        drow = dv_ref[...].astype(f32).reshape(1, D)
        for g in range(NG):
            par[g] = jnp.broadcast_to(drow[:, lanes(g)], (8, 128))
        eye = (jax.lax.broadcasted_iota(jnp.int32, (128, 128), 0)
               == jax.lax.broadcasted_iota(jnp.int32, (128, 128), 1))
        brow = bsp_ref[...].astype(f32).reshape(1, S)
        for t in range(S // 128):
            row = jnp.broadcast_to(brow[:, t * 128:(t + 1) * 128], (128, 128))
            col = jnp.sum(jnp.where(eye, row, 0.0), axis=1, keepdims=True)
            bcol[t * 128:(t + 1) * 128, :] = jnp.broadcast_to(col, (128, 128))

    if MAN == 1:
        setup2()

    hp = P // 2
    dep = {"rv": None, "out": [], "keep": None}

    def rel(x, on=None):
        if dep["rv"] is None or not (REL if on is None else on):
            return x
        return jnp.where(dep["keep"], x, dep["rv"])

    def done(x, lag=LAG):
        if dep["rv"] is not None:
            dep["out"].append((lag, x))

    def rel2(x):
        if dep["rv"] is None or not LREL:
            return x
        return jnp.concatenate(
            [jnp.concatenate([rel(x[r:r + 8, 0:128], 1), x[r:r + 8, 128:]], 1)
             for r in range(0, x.shape[0], 8)], 0)

    def done2(xp):
        for r in range(0, xp.shape[0], 8):
            for j in range(0, xp.shape[1] // 128, LDN):
                done(_f(xp[r:r + 8, j * 128:(j + 1) * 128]), LLAG)

    class Stage:
        def __init__(self, g, g0, h, base, base2=None):
            self.g, self.g0, self.h, self.base = g, g0, h, base
            self.base2 = base if base2 is None else base2
            self.early = isinstance(g, int) and g < MIG

        def uh(self, h):
            if h == 0:
                return w, self.base + band(self.g0)
            return uhh, (self.g0 % 2) * 48

        def yb(self, arr, t, pers):
            if pers:
                return self.base + band(self.g0) + OY + arr * 9 + (t - 7)
            return self.base + YT + (self.g0 % 2) * 27 + arr * 9 + (t + 1)

        def kv(self, b):
            if self.h == 0:
                return kvs[self.g % 3], (slice(b * hp, (b + 1) * hp), slice(None))
            return kvh, (self.g, slice(b * hp, (b + 1) * hp), slice(None))

        def dft(self, lo, n):
            return _unpack(dft_p[lo // 2:(lo + n) // 2, :])

    def h_mm(sa, b, h3):
        t0 = (sa.h * HB + b) * P
        hkb = r2[lanes(sa.g), 2 * D + t0:2 * D + t0 + P]
        dft = sa.dft
        if h3:
            return jnp.concatenate(
                [_dot_nt(dft(2 * P, 192), hkb), _dot_nt(dft(2 * P + 192, 192), hkb)], 0)
        c, d = _dot_nt(dft(0, P), hkb), _dot_nt(dft(P, P), hkb)
        return jnp.concatenate([c, d - c, c + d], 0)

    def h_store(sa, b, hd, lo, n):
        ref, o = sa.uh(sa.h)
        ref[o + (3 + lo // P) * 8 + b, lo % P:lo % P + n, :] = _pack(hd[lo:lo + n])

    def kv_make(sa, b, nb):
        cols = lanes(sa.g)
        t0 = (sa.h * HB + b) * P
        n = nb * P
        taps = par[sa.g]
        if t0 == 0:
            kf_s[0:8, :] = jnp.zeros((8, 128), f32)
        elif b == 0:
            kf_s[0:8, :] = r2[t0 - 16:t0, cols].astype(f32)[8:16]
        l0 = b * P + 8
        kf_s[l0:l0 + n, :] = r2[t0:t0 + n, cols].astype(f32)
        ks = kf_s[l0:l0 + n, :] * taps[0:1]
        for j in range(1, 4):
            ks = ks + kf_s[l0 - j:l0 - j + n, :] * taps[j:j + 1]
        kv = _pack((ks * r2[t0:t0 + n, lanes(sa.g, D)].astype(f32)).astype(bf16))
        for j in range(nb):
            ref, idx = sa.kv(b + j)
            ref[idx] = kv[j * hp:(j + 1) * hp]

    def kv_fine(sa, b, q, nq):
        cols = lanes(sa.g)
        n = P // nq
        t0 = (sa.h * HB + b) * P + q * n
        l0 = b * P + q * n + 8
        if t0 == 0:
            kf_s[0:8, :] = jnp.zeros((8, 128), f32)
        elif l0 == 8:
            kf_s[0:8, :] = r2[t0 - 16:t0, cols].astype(f32)[8:16]
        kf_s[l0:l0 + n, :] = r2[t0:t0 + n, cols].astype(f32)
        tb = sa.base + band(sa.g0) + OT
        ks = None
        for j in range(4):
            tj = jnp.concatenate([rel(_f(w[tb, 8 * j:8 * j + 8, :]))] * (n // 8), 0)
            term = kf_s[l0 - j:l0 - j + n, :] * tj
            ks = term if ks is None else ks + term
        kv = _pack((ks * r2[t0:t0 + n, lanes(sa.g, D)].astype(f32)).astype(bf16))
        o = (b * P + q * n) // 2
        if sa.h:
            kvh[sa.g, o:o + n // 2, :] = kv
        else:
            kvs[sa.g % 3][o:o + n // 2, :] = kv
        for j in range(n // 16):
            done(_f(kv[8 * j:8 * j + 8]))

    def u_mm(sa, b):
        ref, idx = sa.kv(b)
        kvb = _unpack(ref[idx])
        return _dot(sa.dft(0, P), kvb), _dot(sa.dft(P, P), kvb)

    def u_store(sa, b, u, rr):
        ref, o = sa.uh(sa.h)
        for a in range(2):
            ref[o + a * 8 + b, rr, :] = _pack(u[a][rr])
        ref[o + 16 + b, rr, :] = _pack(u[0][rr] + u[1][rr])

    def c_prep(sb, sp, dup, bs=range(HB)):
        pers = sb.h == 1
        r = slice(sp * 16, sp * 16 + 16)
        pk = slice(sp * 8, sp * 8 + 8)
        pk2 = slice(hp + sp * 8, hp + sp * 8 + 8)

        def ld(t):
            s1, s3, s2 = (_f(w[sb.yb(a, t, pers), r, :]) for a in range(3))
            s1 = jnp.concatenate([rel(s1[0:8]), rel(s1[8:16])], 0)
            return s1 - s3, s1 + s2

        t0 = sb.h * HB + bs[0]
        prev = ld(t0 - 1) if t0 else None
        for b in bs:
            t = sb.h * HB + b
            cr, ci = ld(t)
            if prev is None:
                a, c = cr, ci
            elif sp < 4:
                a, c = cr - prev[1], ci + prev[0]
            else:
                a, c = cr + prev[1], ci - prev[0]
            prev = (cr, ci)
            a, c = _pack(a.astype(bf16)), _pack(c.astype(bf16))
            n = (sb.g0 % 2) * HB + b
            cbuf[n, pk, :] = a
            cbuf[n, pk2, :] = c
            done(_f(a))
            done(_f(c))

    def c_mm(sc, b, tok=None):
        dft = sc.dft
        n = (sc.g0 % 2) * HB + b
        a, c = _unpack(cbuf[n, 0:hp, :]), _unpack(cbuf[n, hp:P, :])
        yt = _dot(dft(5 * P, P), a) + _dot(dft(6 * P, P), c)
        if tok:
            yt = tok(yt)
        ref, idx = sc.kv(b)
        kv = _unpack(ref[idx]).astype(f32)
        return (yt + kv * par[sc.g][4:5]).astype(bf16)

    def c_store(sc, b, y):
        t0 = (sc.h * HB + b) * P
        y_v[t0:t0 + P, lanes(sc.g)] = y

    def b_terms(sb, sl, arr, terms, init):
        r = slice(sl * 8, sl * 8 + 8)
        ha, ua = [(0, 2), (2, 1), (1, 0)][arr]
        out, hs, us, seen = {}, {}, {}, set()
        for t, uh_, b, hh_, d in terms:
            if t not in out and init(t):
                out[t] = _f(w[sb.yb(arr, t, True), r, :])
            if (hh_, d) not in hs:
                hr, ho = sb.uh(hh_)
                hs[hh_, d] = _f(hr[ho + (3 + ha) * 8 + d, r, :])
                if REL == 2:
                    hs[hh_, d] = rel(hs[hh_, d])
            if (uh_, b) not in us:
                ur, uo = sb.uh(uh_)
                us[uh_, b] = _f(ur[uo + ua * 8 + b, r, :])
            term = hs[hh_, d] * us[uh_, b]
            if t not in seen and REL == 1:
                term = rel(term)
            seen.add(t)
            out[t] = out[t] + term if t in out else term
        for t, val in out.items():
            done(val)
            if t <= 7:
                w[sb.yb(arr, t, False), r, :] = _pack(val)
            if t >= 7:
                w[sb.yb(arr, t, True), r, :] = _pack(val)

    def mk_terms(ts, sets, bs=range(8)):
        return [(t, uh_, b, hh_, t - 8 * uh_ - 8 * hh_ - b) for uh_, hh_ in sets for t in ts
                for b in bs if 0 <= t - 8 * uh_ - 8 * hh_ - b <= 7]

    def b_slice(sb, sl, kind, split=False):
        ab = [(1, 0), (0, 1)]
        if kind == "lo":
            groups = [(mk_terms(range(0, 8), [(0, 0)]), lambda t: False)]
        elif kind == "mi":
            groups = [(mk_terms(range(8, 15), [(0, 0)]), lambda t: False)]
        elif not split or BM == "pass":
            groups = [(mk_terms(range(8, 16), ab), lambda t: t < 15)]
        elif BM == "q4" and MI == 2 and not sb.early:
            ll = [(0, 0)]
            groups = [(mk_terms(range(8, 10), ll + ab), lambda t: False),
                      (mk_terms(range(10, 12), ll + ab), lambda t: False),
                      (mk_terms(range(12, 16), ab[:1], range(0, 4)), lambda t: False),
                      (mk_terms(range(12, 16), ab[1:], range(0, 4)), lambda t: True),
                      (mk_terms(range(12, 16), ll + ab, range(4, 8)), lambda t: True)]
        elif BM == "q4":
            groups = [(mk_terms(range(8, 12), ab), lambda t: True),
                      (mk_terms(range(12, 16), ab[:1], range(0, 4)), lambda t: t < 15),
                      (mk_terms(range(12, 16), ab[1:], range(0, 4)), lambda t: True),
                      (mk_terms(range(12, 16), ab, range(4, 8)), lambda t: True)]
        else:
            groups = [(mk_terms(range(8, 16), ab[:1]), lambda t: t < 15),
                      (mk_terms(range(8, 16), ab[1:]), lambda t: True)]
        fs = [lambda arr=arr, g=g: b_terms(sb, sl, arr, *g) for g in groups for arr in range(3)]
        if split:
            return fs
        for f in fs:
            f()

    def static_stage(s, zi):
        if s < 0 or s >= 2 * NG:
            return None
        if PREPIN == 0:
            return Stage(s % NG, s % NG, s // NG, 0)
        return Stage(s % NG, s % NG, s // NG, zab[min(zi, 1)], zab[0])

    def conv_pieces(sa, sb, sc, frac=1.0, h3=0, kq=KQ, psp=PSP):
        def hu(b, tok):
            hd = h_mm(sa, b, h3)
            u = u_mm(sa, b)
            u = (tok(u[0]), u[1])
            for a in range(3):
                h_store(sa, b, hd, a * P, P)
            u_store(sa, b, u, slice(0, P))

        def cc(b, tok):
            ys = [c_mm(sc, b + j, tok if j == 0 else None) for j in range(2)]
            for j in range(2):
                c_store(sc, b + j, ys[j])

        mx, out = [], []
        d = 1.0 / (HB + 1.0)
        for b in range(HB):
            if sa:
                kvp = [lambda b=b, q=q: kv_fine(sa, b, q, kq) for q in range(kq)]
                mx.append(((b + 1.2) * d, lambda tok, b=b: hu(b, tok), kvp))
                out += [((b + q / kq) * d, 200 / kq, f) for q, f in enumerate(kvp)]
            if sc and b % 2 == 0:
                mx.append((b / HB * frac, lambda tok, b=b: cc(b, tok), []))
        if sb:
            for sl in range(2 * HB):
                fs = b_slice(sb, sl, "hi", True) if sb.h else (
                    b_slice(sb, sl, "lo", True) + ([] if MI and not sb.early else b_slice(sb, sl, "mi", True)))
                fs = [((432.0 if MI < 2 or sb.early else CH if sb.h else CL) / len(fs), f) for f in fs]
                if sl % 2:
                    fs = fs + [(130 / psp, lambda sl=sl, bs=bs: c_prep(sb, sl // 2, True, bs))
                               for bs in _spread(list(range(HB)), psp)]
                for j, (c_, f) in enumerate(fs):
                    out.append(((sl + j / len(fs)) / (2.0 * HB), c_, f))
        return sorted(mx, key=lambda x: x[0]), sorted(out, key=lambda x: x[0])

    def scheduler(wts, pieces, rpt, lag):
        cum = np.cumsum(wts) / np.sum(wts)
        slots = [[] for _ in wts]
        tot, run = sum(c_ for _, c_, _ in pieces), 0.0
        for _, c_, f in pieces:
            slots[min(int(np.searchsorted(cum, run / tot, side="right")), len(wts) - 1)].append(f)
            run += c_
        pend, cnt, ran = [], [0], []
        keep = jnp.full((8, 128), zs[5], jnp.int32) == 0

        def call(f):
            if not any(f is g for g in ran):
                ran.append(f)
                f()

        def need(fs):
            for f in fs:
                call(f)

        def tok(val):
            if not pieces:
                return val
            tiles = [val[r0:r0 + 8] for r0 in range(0, val.shape[0], 8)]
            for r0 in range(0, val.shape[0], rpt):
                due = [v for n, v in pend if n <= cnt[0]]
                pend[:] = [e for e in pend if e[0] > cnt[0]]
                for j, v in enumerate(due):
                    q = r0 // 8 + j % (rpt // 8)
                    tiles[q] = jnp.where(keep, tiles[q], v)
                dep["rv"], dep["out"], dep["keep"] = val[r0:r0 + 8], [], keep
                for f in slots[cnt[0]]:
                    call(f)
                pend.extend((cnt[0] + lag, v) for _, v in dep["out"])
                dep["rv"] = None
                cnt[0] += 1
            return jnp.concatenate(tiles, 0)

        return tok, need

    for s in range(NG + 2):
        if SPL0 and s == 0:
            wait(lo0(0))
        elif s == 1 and BPRE:
            pass
        elif not (NOW & 1 and s > 0 or NOW & 4):
            wait(grp_copies(s % NG, s // NG))
        start(sched.get(s, []))
        if MAN == 2 and s == 0:
            wait(small[1:3])
            setup2()
        if ONLY:
            continue
        mx, pieces = conv_pieces(static_stage(s, 0), static_stage(s - 1, 1),
                                 static_stage(s - 2, 2), h3=H3PRE, kq=KQ0, psp=PSP0)
        if s == 1 and BPRE:
            kvp = [f for e in mx for f in e[2]]
            bp = [e for e in pieces if not any(e[2] is f for f in kvp)]
            bp = bp[:int(len(bp) * BPRE)]
            for e in bp:
                e[2]()
            pieces = [e for e in pieces if not any(e is x for x in bp)]
            wait(grp_copies(1, 0))
        if SPL0 and s == 0:
            pieces = []
        tok, need = scheduler([1.0] * (len(mx) * P // RPT0), pieces, RPT0, LAG0)
        for j, (_, f, pre) in enumerate(mx):
            if SPL0 and s == 0 and j == SPL0:
                wait(lo0(1))
            need(pre)
            f(tok)

    npc = TM // PR

    def rows_of(i, r0=0, nr=TM):
        return pl.ds(pl.multiple_of(i * TM + r0, PR), nr)

    def a_layer_piece(r, i, iy, ps, stage_c):
        if not ps:
            return
        rr = rows_of(i, ps[0] * PR, len(ps) * PR)
        ry = rows_of(iy, ps[0] * PR, len(ps) * PR)
        x = r[rr, XC:XC + D].astype(f32)
        x = x + _ln(x) * y_v[ry, 0:D].astype(f32)
        r[rr, XC:XC + D] = x.astype(bf16)
        if stage_c is None:
            xnl[ps[0] * PR // 2:(ps[-1] + 1) * PR // 2, 0:D] = _pack(_ln(x).astype(bf16))
        else:
            r[rr, stage_c:stage_c + D] = _ln(x).astype(bf16)

    def norm_piece(r, i, ps):
        if not ps:
            return
        rr = rows_of(i, ps[0] * PR, len(ps) * PR)
        r[rr, FH:F] = _ln(r[rr, FH:F].astype(f32)).astype(bf16)

    nzh = FH // TN
    noc = D // TN

    def z_chunk(r, i, c, tn=TN, tok=lambda v: v, ks=1):
        cs = slice(c * tn, (c + 1) * tn)
        kk = D // ks
        acc = None
        for k in range(ks):
            part = _dot(_unpack(xnl[:, k * kk:(k + 1) * kk]), win_v[k * kk:(k + 1) * kk, cs])
            if tn > 128 and ks > 1:
                part = jnp.concatenate([tok(part[:, 0:128]), part[:, 128:]], 1)
            else:
                part = tok(part)
            acc = part if acc is None else acc + part
        r[rows_of(i), cs] = _gelu(acc).astype(bf16)

    def g_chunk(r, i, c, side=None):
        cs = slice(c * TN, (c + 1) * TN)
        rr = rows_of(i)
        ks = KG if side else 1
        kk = S // ks
        gg = None
        for k in range(ks):
            if side:
                for f in side[c * ks + k]:
                    f()
            part = _dot(wsp_v[rr, k * kk:(k + 1) * kk],
                        r[k * kk:(k + 1) * kk, FH + c * TN:FH + (c + 1) * TN])
            gg = part if gg is None else gg + part
            if side:
                tk = gg[0:16, 0:128] if TKF else gg[TM - 16:TM, TN - 128:TN]
                r2[S:S + 16, 0:128] = tk.astype(bf16)
        bb = bcol[rr, :]
        gg = gg + jnp.concatenate([bb] * (TN // 128), axis=1)
        ml[:, cs] = _pack((r[rr, cs].astype(f32) * gg).astype(bf16))

    def o_chunk(src, dst, dst_c, i, c):
        cs = slice(c * TN, (c + 1) * TN)
        rr = rows_of(i)
        o = _dot(_unpack(ml[:, 0:FH]), wout_v[:, cs])
        x = src[rr, XC + c * TN:XC + (c + 1) * TN].astype(f32) + o
        dst[rr, dst_c + c * TN:dst_c + (c + 1) * TN] = x.astype(bf16)

    parts_z = _spread(list(range(npc)), nzh)
    parts_o = _spread(list(range(npc)), noc)

    def finish(pending):
        wait(pending)
        out_copy(NR - 1).start()
        out_copy(NR - 1).wait()

    late = sum([hi(g) for g in range(4, NG)], []) + [q_copy(i) for i in range(2, NR)]
    if not LATE:
        start(late)
    if not NOW & 2:
        q_copy(0).wait()
    for ps in parts_z:
        a_layer_piece(r1, 0, 0, ps, 0)
    if not NOW & 2:
        wait(win_copy if W1 == 0 else win_copy[:1])
    if STOP == 1:
        finish([c for g in range(2, NG) for c in grp_copies(g, 1)] + [q_copy(i) for i in range(1, NR)])
        return
    if not LATE:
        start([wsp_copy, wout_copy])

    def ln_pieces(fn, lo=0.0, hi=1.0, n=LNP, sub=None):
        d = (hi - lo) / n
        return [(lo + j * d, lambda ps=ps: fn(ps))
                for j, ps in enumerate(_spread(sub or list(range(npc)), n))]

    def p1_half(i, hh, lnp, conv=((), ()), hook=None):
        mx, pieces = conv
        if NOLN & (1 << hh) and pieces:
            lnp = []
        tn = TN1 if pieces else TNC
        nz1 = FH // tn
        ks = 2 * tn // 128
        rpt = TM // TPS
        grp = [[e for e in mx if min(int(e[0] * nz1 + 1e-6), nz1 - 1) == c] for c in range(nz1)]
        wts = []
        for c in range(nz1):
            wts += [WC] * (len(grp[c]) * P // rpt) + [1.0] * (TPS * (ks - 1)) + [W0] * TPS
        tok, need = scheduler(wts, pieces, rpt, LAG)
        for c in range(nz1):
            if hook and c and (hh, c * tn // 128) in wpc:
                hook(wpc[hh, c * tn // 128].wait)
            for p_, f in lnp:
                if min(int(p_ * nz1 + 1e-6), nz1 - 1) == c:
                    f()
            for _, f, pre in grp[c]:
                need(pre)
                f(tok)
            z_chunk(r1, i, c + (nz1 if hh == 0 else 0), tn, tok, ks if pieces else 1)

    def p1a_body(i, carry, first=None):
        def once(f):
            if first is None:
                pl.when(i == 0)(f)
            elif first:
                f()

        hk0 = hk1 = once if first is not False else None
        i0 = i
        if TRA:
            i = jnp.minimum(i, 2)

            @pl.when(i0 < 3)
            def _():
                q_copy(i + 1).wait()
                wait(grp_copies(2 * i + 2, 1))
        elif not NOW & 2:
            q_copy(i + 1).wait()
            wait(grp_copies(2 * i + 2, 1))
        if W1 < 2:
            wait(grp_copies(2 * i + 3, 1))
        base = i * PB

        def st(g0):
            sg = Stage(2 * i + g0, g0, 1, base)
            sg.early = bool(first) and g0 < MIG
            return sg

        xnl[:, 0:D] = _pack(r1[rows_of(i), 0:D])
        al = lambda ps: a_layer_piece(r1, i + 1, i + 1, ps, 0)
        h0, h1 = list(range(npc // 2)), list(range(npc // 2, npc))
        p1_half(i, 0, ln_pieces(al, n=LNH, sub=h0) if DEFN == 2 else ln_pieces(al, n=LNA),
                conv_pieces(st(2), st(1), st(0)), hk0)
        if TRA:
            @pl.when(i0 < 3)
            def _():
                wait(grp_copies(2 * i + 3, 1))
        elif W1 >= 2 and not NOW & 2:
            wait(grp_copies(2 * i + 3, 1))
        if W1 == 2:
            def mid():
                win_copy[1].wait()
                start(late)

            once(mid)
        p1_half(i, 1, [ln_pieces(lambda ps: norm_piece(r1, i, ps), n=LNA), [],
                       ln_pieces(al, n=LNH, sub=h1)][DEFN],
                conv_pieces(st(3), st(2), st(1)), hk1)
        return carry

    if ONLY != 'p1c':
        if WQ == 2:
            p1a_body(zs[13], 0, True)
            jax.lax.fori_loop(1, 3, lambda i, cr: p1a_body(i, cr, False), 0)
        else:
            jax.lax.fori_loop(0, zs[14] if TRA else 3, p1a_body, 0)
    else:
        wait([q_copy(i) for i in range(1, 4)] + [c for g in range(2, NG) for c in grp_copies(g, 1)])

    if W1 in (1, 3):
        win_copy[1].wait()
    if LATE:
        start([wsp_copy, wout_copy])
    if NOW & 2:
        wait(win_copy + [q_copy(i) for i in range(4)] + sum([hi(g) for g in range(2, NG)], []))
    if NOW & 5:
        wait(sum([list(grp_copies(s % NG, s // NG)) for s in range(0 if NOW & 4 else 1, NG + 2)], []))
    wait([q_copy(i) for i in range(4, NR)])
    if ONLY == 'p1a':
        finish([wsp_copy, wout_copy])
        return
    i3 = zs[8]
    xnl[:, 0:D] = _pack(r1[rows_of(i3), 0:D])
    if DYNB:
        b3 = zs[9]
        s14, s15 = Stage(2 * i3, 0, 1, b3), Stage(2 * i3 + 1, 1, 1, b3)
    else:
        s14, s15 = static_stage(14, 0), static_stage(15, 0)
    p1_half(i3, 0, [], conv_pieces(None, s15, s14))
    p1_half(i3, 1, ([] if DEFN else ln_pieces(lambda ps: norm_piece(r1, i3, ps), 0.0, 0.5, 4))
            + ln_pieces(lambda ps: a_layer_piece(r1, i3 + 1, i3 + 1, ps, 0), 0.45, 1.0, 4),
            conv_pieces(None, None, s15, 0.4))

    def p1c_body(i, carry):
        iy = jnp.minimum(i + 1, NR - 1)
        xnl[:, 0:D] = _pack(r1[rows_of(i), 0:D])
        p1_half(i, 0, ln_pieces(lambda ps: a_layer_piece(r1, i + 1, iy, ps, 0)))
        p1_half(i, 1, ln_pieces(lambda ps: norm_piece(r1, i, ps))
                + (ln_pieces(lambda ps: norm_piece(r1, i - 4, ps)) if DEFN else []))
        return carry

    if U1 == 1:
        jax.lax.fori_loop(4, zs[11] if TR1 else NR, p1c_body, 0)
    else:
        jax.lax.fori_loop(2, 4, lambda j, cr: p1c_body(2 * j + 1, p1c_body(2 * j, cr)), 0)

    wsp_copy.wait()
    wout_copy.wait()
    if STOP == 2:
        finish([])
        return

    last = NR - 1
    parts_a = _spread(list(range(npc)), NA2) + [[]] * (nzh - NA2)

    def g_side(i, ia, inorm):
        pp = [list(range(j, j + PG)) for j in range(0, npc, PG)]
        base = ia * TM

        def rws(ps, off=0):
            return pl.ds(pl.multiple_of(base + (off + ps[0] * PR), PR), len(ps) * PR)

        def cp(ps):
            xnl[ps[0] * PR // 2:(ps[-1] + 1) * PR // 2, 0:D] = _pack(r2[rws(ps), FH:FH + D])

        def a2a(ps):
            rr = rws(ps)
            x = r2[rr, XC:XC + D].astype(f32)
            r2[rr, XC:XC + D] = (x + _ln(x) * y_v[rr, 0:D].astype(f32)).astype(bf16)

        def a2b(ps):
            rr = rws(ps)
            r2[rr, FH:FH + D] = _ln(r2[rr, XC:XC + D].astype(f32)).astype(bf16)

        def nrm(ps):
            rr = rws(ps, -TM)
            r2[rr, FH:F] = _ln(r2[rr, FH:F].astype(f32)).astype(bf16)

        nw = nzh * KG
        seq = []
        for j, ps in enumerate(pp):
            seq.append([lambda ps=ps: a2a(ps)])
            if j:
                seq[-1].insert(0, lambda ps=pp[j - 1]: cp(ps))
            if inorm is not None:
                seq.append([lambda ps=ps: nrm(ps)])
            seq.append([lambda ps=ps: a2b(ps)])
        seq.append([lambda: cp(pp[-1])])
        side = [sum(x, []) for x in _spread(seq, nw - NA2)] + [[]] * NA2
        for c in range(nzh):
            g_chunk(r1, i, c, side)

    def p2r_body(i, carry):
        for c in range(nzh):
            z_chunk(r2, i - 1, nzh + c)
        for c in range(noc):
            o_chunk(r1, r2, XC, i, c)
        for c in range(nzh):
            z_chunk(r2, i - 1, c)
        g_side(i + 1, i, i - 1)
        return carry

    if ROT:
        for c in range(nzh):
            g_chunk(r1, 0, c)
        for c in range(noc):
            o_chunk(r1, r2, XC, 0, c)
        g_side(1, zs[13], None)
        jax.lax.fori_loop(1, NR - 1, p2r_body, 0)
        i7 = zs[12]
        for c in range(nzh):
            z_chunk(r2, i7 - 1, nzh + c)
        for c in range(noc):
            if EPI & 1:
                norm_piece(r2, i7 - 1, parts_o[c])
            o_chunk(r1, r2, XC, i7, c)
        for c in range(nzh):
            a_layer_piece(r2, i7, i7, parts_z[c], FH)
            z_chunk(r2, i7 - 1, c)
        xnl[:, 0:D] = _pack(r2[rows_of(last), FH:FH + D])
        for c in range(nzh):
            if not EPI & 1:
                norm_piece(r2, i7 - 1, parts_z[c])
            z_chunk(r2, i7 if EPI & 4 else last, nzh + c)
        for c in range(nzh):
            norm_piece(r2, i7 if EPI & 2 else last, parts_z[c])
            z_chunk(r2, i7 if EPI & 4 else last, c)
    else:
        for c in range(nzh):
            g_chunk(r1, 0, c)
        for c in range(noc):
            o_chunk(r1, r2, XC, 0, c)
        for ps in parts_z:
            a_layer_piece(r2, 0, 0, ps, FH)

        def p2_body(i, carry):
            xnl[:, 0:D] = _pack(r2[rows_of(i - 1), FH:FH + D])
            for c in range(nzh):
                g_chunk(r1, i, c)
            for c in range(nzh):
                z_chunk(r2, i - 1, nzh + c)
            for c in range(noc):
                norm_piece(r2, i - 1, parts_o[c])
                o_chunk(r1, r2, XC, i, c)
            for c in range(nzh):
                a_layer_piece(r2, i, i, parts_z[c], FH)
                z_chunk(r2, i - 1, c)
            return carry

        if U2 == 1:
            jax.lax.fori_loop(1, zs[10] if TR2 else NR, p2_body, 0)
        else:
            jax.lax.fori_loop(0, 3, lambda j, cr: p2_body(2 * j + 2, p2_body(2 * j + 1, cr)), 0)
            p2_body(zs[12], 0)

        last = NR - 1
        xnl[:, 0:D] = _pack(r2[rows_of(last), FH:FH + D])
        for c in range(nzh):
            z_chunk(r2, last, nzh + c)
        for c in range(nzh):
            norm_piece(r2, zs[12] if EPI & 2 else last, parts_z[c])
            z_chunk(r2, last, c)

    for c in range(nzh):
        g_chunk(r2, 0, c)

    def p3_body(i, carry):
        for c in range(noc):
            o_chunk(r2, y_v, 0, i - 1, c)
        out_copy(i - 1).start()
        for c in range(nzh):
            g_chunk(r2, i, c)
        return carry

    if U3 == 1:
        jax.lax.fori_loop(1, NR, p3_body, 0)
    elif U3 == 2:
        jax.lax.fori_loop(0, 3, lambda j, cr: p3_body(2 * j + 2, p3_body(2 * j + 1, cr)), 0)
        p3_body(NR - 1, 0)
    else:
        for i in range(1, NR):
            p3_body(i, 0)
    def out_last(c):
        cs = slice(c * TN, (c + 1) * TN)
        return pltpu.make_async_copy(y_v.at[blk(last), cs], out_hbm.at[0, blk(last), cs],
                                     sem_o.at[NR + c])

    for c in range(noc):
        o_chunk(r2, y_v, 0, NR - 1, c)
        if OSP:
            out_last(c).start()
    if not OSP:
        out_copy(NR - 1).start()
    for i in range(NR - OSP):
        out_copy(i).wait()
    if OSP:
        wait([out_last(c) for c in range(noc)])


@jax.jit
def pallas_interleave_layers__ssm_conv_h3__mixer_gmlp__prompt_kernel(
    A_q, A_k, A_v, A_shift_k, A_ssm_k, A_ssm_D, B_x, B_w_in, B_w_sp, B_b_sp, B_w_out,
):
    del B_x
    anyspec = pl.BlockSpec(memory_space=pl.ANY)
    vmem = pl.BlockSpec(memory_space=pltpu.VMEM)
    return pl.pallas_call(
        _kernel,
        grid=(1,),
        in_specs=[anyspec] * 11,
        out_specs=anyspec,
        out_shape=jax.ShapeDtypeStruct((1, S, D), bf16),
        scratch_shapes=[
            pltpu.VMEM((D, F + PS3), bf16),
            pltpu.VMEM((S, S + PS1), bf16),
            pltpu.VMEM((FH, D + PS2), bf16),
            pltpu.VMEM((S, D + PS5), bf16),
            pltpu.VMEM((S + TM, RW), bf16),
            pltpu.VMEM((S + 16, RW), bf16),
            pltpu.VMEM((TM // 2, D + PS4), u32),
            pltpu.VMEM((TM // 2, FH + PS6), u32),
            pltpu.VMEM((NTW, P + PADW, 128), u32),
            pltpu.VMEM((96, P + PADW, 128), u32),
            pltpu.VMEM((HS // 2, 128), u32),
            pltpu.VMEM((HS // 2, 128), u32),
            pltpu.VMEM((HS // 2, 128), u32),
            pltpu.VMEM((NG, HS // 2, 128), u32),
            pltpu.VMEM((2 * HB, P + PADW, 128), u32),
            pltpu.VMEM((HS + 8, 128), f32),
            pltpu.VMEM((7 * P // 2, 128), u32),
            pltpu.VMEM((S, 128), f32),
            pltpu.VMEM((NG, 8, 128), f32),
            pltpu.SMEM((16,), jnp.int32),
            pltpu.VMEM((4, D), bf16),
            pltpu.VMEM((D,), bf16),
            pltpu.VMEM((S,), bf16),
            pltpu.VMEM((7 * P, 128), bf16),
            pltpu.SemaphoreType.DMA((2 * NG,)),
            pltpu.SemaphoreType.DMA((2 * NG,)),
            pltpu.SemaphoreType.DMA((2 * NG,)),
            pltpu.SemaphoreType.DMA((16,)),
            pltpu.SemaphoreType.DMA((NR,)),
            pltpu.SemaphoreType.DMA((NR + 4,)),
            pltpu.SemaphoreType.DMA((7,)),
        ],
        compiler_params=pltpu.CompilerParams(
            dimension_semantics=("arbitrary",),
            vmem_limit_bytes=124 * 1024 * 1024,
        ),
    )(A_q, A_k, A_v, A_shift_k.T, A_ssm_k, A_ssm_D, B_w_in, B_w_sp, B_b_sp, B_w_out,
      _dft_constants())
```

```python
import numpy as np
import jax
import jax.numpy as jnp
import jax.experimental.pallas as pl
import jax.experimental.pallas.tpu as pltpu

S = 2048
D = 1024
F = 3584
FH = F // 2
P = 128
NB = S // P
HB = NB // 2
HS = S // 2
NG = D // 128
TM = 256
NR = S // TM
TN = 256
PR = 16
XC = F
RW = F + D
NT = FH // 128
EPS = 1e-5

STOP = 0
H3PRE = 0
MIG = 1
WCC = 1.0
CG = 4
HG = 1
COF = 0
TH0 = 1
TH1 = 1
ORS = 128
ZRS = 0
ZNP = 2
P2O = 0
DNS = 0
PREPIN = 0
KS = 2
TPS = 8
W0 = 0.8
LNP = 7
LND = 2
TN1 = 128
BM = 'q4'
ONLY = ''
XTOK = 1
PSP = 3
KQ = 4
WC = 1.0
LAG = 2
REL = 0
LLAG = 8
LREL = 0
LDN = 1
LNM = 0
HARD = 1
ALT = 1
NOLN = 0
KQ0 = 2
PSP0 = 2
RPT0 = 16
LAG0 = 2
TNC = 256
LNA = 7
H3P1 = 0
ORDER = "H0 lo0 H1 mi0 H2 lo1 C0 mi1 P0 U0 lo2 mi2 U1 lo3 C1 mi3 P1".split()
P1ORD = 'CUHPKB'
W1 = 2
DORD = 3
DYNB = 1
NOW = 0
MAN = 2
SPL0 = 0
BPRE = 0.15
MI = 2
WQ = 2
PAIR = 0
WB0 = '0 7 14'.split()
WB1 = '0 7 14'.split()
WST = '2 5 7 9'.split()
DW2 = 5
DW3 = 7
DW4 = 9
WQC = 7
CH = 500
CL = 250
LN1 = 0
PADW = 8
PS1 = 0
PS2 = 128
PS5 = 0
PS6 = 0
PS3 = 0
PS4 = 0
EPI = 0
KG = 4
PG = 2
ROT = 0
TRA = 0
NA2 = 2
TKF = 0
DEFN = 2
LNH = 5
U2 = 1
U1 = 1
OSP = 1
U3 = 2
TR2 = 0
TR1 = 0
TINY = 0
LATE = 1

BS = 76
OY = 48
OT = 75
OO = 58
OK_ = 66
PB = 2 * BS
OD = 2 * BS
YT = 4 * PB
TK = YT + 54
NTW = TK
Z1 = 0
Z2 = Z1 + NT * NR
YV = Z2 + NT * (NR + 1)
NTZ = YV + NR * NG


def band(n):
    return n * BS


f32 = jnp.float32
bf16 = jnp.bfloat16
u32 = jnp.uint32


def _dft_constants():
    n = np.arange(P)
    k = np.concatenate([np.arange(0, P, 2), P - 1 - np.arange(0, P, 2)])
    ang = 2.0 * np.pi * np.outer(2 * k + 1, n) / (4 * P)
    fre, fim = np.cos(ang), -np.sin(ang)
    gi = np.concatenate([fre[:P // 2].T, fim[:P // 2].T], 1) / P
    g = np.concatenate([gi[0::2], gi[1::2]], 0)
    return jnp.asarray(np.concatenate([fim, fre + fim, fre, fim - fre, g], 0), dtype=bf16)


def _ln(x):
    m = jnp.mean(x, axis=-1, keepdims=True)
    if LN1:
        v = jnp.maximum(jnp.mean(x * x, axis=-1, keepdims=True) - m * m, 0.0)
        return (x - m) * jax.lax.rsqrt(v + EPS)
    xc = x - m
    v = jnp.mean(xc * xc, axis=-1, keepdims=True)
    return xc * jax.lax.rsqrt(v + EPS)


def _gelu(z):
    c = 0.7978845608028654
    u = z * (c + (c * 0.044715) * (z * z))
    h = 0.5 * z
    return h + h * jnp.tanh(u)


def _dot(a, b):
    return jnp.dot(a, b, preferred_element_type=f32)


def _spread(work, n):
    return [work[(j * len(work)) // n:((j + 1) * len(work)) // n] for j in range(n)]


def _dot_nt(a, b):
    return jax.lax.dot_general(a, b, (((1,), (1,)), ((), ())), preferred_element_type=f32)


def _pack(x):
    return pltpu.bitcast(x, u32)


def _unpack(x):
    return pltpu.bitcast(x, bf16)


def _f(x):
    return pltpu.bitcast(x, f32)


def _kernel(q_hbm, k_hbm, v_hbm, shk_hbm, hk_hbm, dv_hbm, win_hbm, wsp_hbm, bsp_hbm,
            wout_hbm, dft_hbm, out_hbm,
            win_v, wsp_v, wout_v, y_v, r1, r2, xnl, ml,
            w, uhh, kv0, kv1, kv2, kvh, cbuf, kf_s, dft_p, bcol, par, zs,
            shk_ref, dv_ref, bsp_ref, dft_ref,
            sem_k, sem_v, sem_h, sem_w, sem_q, sem_o, sem_s):
    small = [pltpu.make_async_copy(a, b, sem_s.at[j]) for j, (a, b) in enumerate(
        [(shk_hbm, shk_ref), (dv_hbm, dv_ref), (bsp_hbm, bsp_ref), (dft_hbm, dft_ref)])]
    for c in (small if MAN == 1 else [small[0], small[3]]):
        c.start()
    def lanes(g, off=0):
        if isinstance(g, int):
            return slice(off + g * 128, off + (g + 1) * 128)
        return pl.ds(pl.multiple_of(off + g * 128, 128), 128)

    def grp_copies(g, h):
        cols, rows = lanes(g), slice(h * HS, (h + 1) * HS)
        s = h * NG + g
        hrows = slice(2 * D + h * HS, 2 * D + (h + 1) * HS)
        if TINY & 1:
            rows = slice(h * HS, h * HS + 128)
            hrows = slice(2 * D + h * HS, 2 * D + h * HS + 128)
        if PAIR and isinstance(s, int) and 2 <= s < NG + 2:
            hc = pltpu.make_async_copy(hk_hbm.at[cols, rows], r2.at[cols, hrows], sem_h.at[s])
            if s % 2:
                return (hc,)
            c2 = slice(g * 128, (g + 2) * 128)
            return (hc, pltpu.make_async_copy(k_hbm.at[0, rows, c2], r2.at[rows, c2], sem_k.at[s]),
                    pltpu.make_async_copy(v_hbm.at[0, rows, c2],
                                          r2.at[rows, D + g * 128:D + (g + 2) * 128], sem_v.at[s]))
        return (pltpu.make_async_copy(hk_hbm.at[cols, rows], r2.at[cols, hrows], sem_h.at[s]),
                pltpu.make_async_copy(k_hbm.at[0, rows, cols], r2.at[rows, cols], sem_k.at[s]),
                pltpu.make_async_copy(v_hbm.at[0, rows, cols], r2.at[rows, lanes(g, D)],
                                      sem_v.at[s]))

    def lo0(part):
        r = slice(0, SPL0 * P) if part == 0 else slice(SPL0 * P, HS)
        hr = slice(2 * D + r.start, 2 * D + r.stop)
        sm = [sem_h.at[0], sem_k.at[0], sem_v.at[0]] if part else [sem_s.at[4 + j] for j in range(3)]
        return [pltpu.make_async_copy(hk_hbm.at[0:128, r], r2.at[0:128, hr], sm[0]),
                pltpu.make_async_copy(k_hbm.at[0, r, 0:128], r2.at[r, 0:128], sm[1]),
                pltpu.make_async_copy(v_hbm.at[0, r, 0:128], r2.at[r, D:D + 128], sm[2])]

    def blk(i):
        if isinstance(i, int):
            return slice(i * TM, (i + 1) * TM)
        return pl.ds(pl.multiple_of(i * TM, TM), TM)

    def q_copy(i):
        return pltpu.make_async_copy(q_hbm.at[0, blk(i), :], r1.at[blk(i), XC:XC + D], sem_q.at[i])

    win_copy = [pltpu.make_async_copy(win_hbm.at[:, FH:F], win_v.at[:, FH:F], sem_w.at[0]),
                pltpu.make_async_copy(win_hbm.at[:, 0:FH], win_v.at[:, 0:FH], sem_w.at[1])]
    wb = [[int(x) for x in WB0], [int(x) for x in WB1]]
    wpc = {}
    for hh_ in range(2):
        for a_, b_ in zip(wb[hh_][:-1], wb[hh_][1:]):
            cs_ = slice((1 - hh_) * FH + a_ * 128, (1 - hh_) * FH + b_ * 128)
            wpc[hh_, a_] = pltpu.make_async_copy(win_hbm.at[:, cs_], win_v.at[:, cs_],
                                                 sem_w.at[4 + len(wpc)])
    win_copy = [wpc[0, 0], wpc[1, 0]]
    wsp_copy = pltpu.make_async_copy(wsp_hbm, wsp_v.at[:, 0:S], sem_w.at[2])
    wout_copy = pltpu.make_async_copy(wout_hbm, wout_v.at[:, 0:D], sem_w.at[3])

    if TINY & 4:
        wsp_copy = pltpu.make_async_copy(wsp_hbm.at[0:16], wsp_v.at[0:16], sem_w.at[2])
        wout_copy = pltpu.make_async_copy(wout_hbm.at[0:16], wout_v.at[0:16], sem_w.at[3])

    def out_copy(i):
        return pltpu.make_async_copy(y_v.at[blk(i), 0:D], out_hbm.at[0, blk(i), :], sem_o.at[i])

    def start(cs):
        for c in cs:
            c.start()

    def wait(cs):
        for c in cs:
            c.wait()

    lo = lambda g: list(grp_copies(g, 0))
    hi = lambda g: list(grp_copies(g, 1))
    if DORD == 0:
        sched = {-1: sum([lo(g) for g in range(NG)], []) + hi(0) + hi(1)
                 + [q_copy(0), q_copy(1), win_copy[0]] + hi(2) + [win_copy[1]] + hi(3)}
    elif DORD == 1:
        sched = {-1: lo(0) + lo(1), 0: lo(2) + lo(3) + lo(4), 1: lo(5) + lo(6) + lo(7),
                 2: hi(0) + hi(1) + [q_copy(0), q_copy(1), win_copy[0]],
                 4: hi(2) + [win_copy[1]] + hi(3)}
    elif DORD == 3:
        sched = {-1: lo(0), -0.5: lo(1), 0: lo(2) + lo(3) + lo(4), 1: lo(5) + lo(6) + lo(7),
                 2: hi(0) + hi(1) + [q_copy(0), q_copy(1), win_copy[0]],
                 4: hi(2) + [win_copy[1]] + hi(3)}
    elif DORD == 4:
        sched = {-1: lo(0), 0: lo(1) + lo(2), 1: lo(3) + lo(4) + lo(5), 2: lo(6) + lo(7) + hi(0) + hi(1),
                 3: [q_copy(0), q_copy(1), win_copy[0]],
                 5: hi(2) + [win_copy[1]] + hi(3)}
    elif DORD == 5:
        sched = {-1: lo(0), -0.5: lo(1), 0: lo(2) + lo(3), 1: lo(4) + lo(5) + [win_copy[0]], 3: lo(6) + lo(7),
                 4: hi(0) + hi(1) + [q_copy(0), q_copy(1)],
                 5: hi(2) + [win_copy[1]] + hi(3)}
    elif DORD == 6:
        sched = {-1: lo(0), -0.5: lo(1), 0: lo(2), 1: lo(3) + lo(4) + lo(5),
                 2: lo(6) + lo(7) + hi(0) + hi(1) + [q_copy(0), q_copy(1), win_copy[0]],
                 4: hi(2) + [win_copy[1]] + hi(3)}
    elif DORD == 2:
        sched = {-1: lo(0) + lo(1) + lo(2), 0: lo(3) + lo(4) + [win_copy[0]], 2: lo(5) + lo(6),
                 3: lo(7) + hi(0) + hi(1) + [q_copy(0), q_copy(1)],
                 5: hi(2) + [win_copy[1]] + hi(3)}
    if WQ:
        sched = {-1: lo(0), -0.5: lo(1), 0: lo(2) + lo(3) + lo(4), 1: lo(5) + lo(6) + lo(7),
                 2: hi(0) + hi(1) + [q_copy(0)]}
        assert len(WST) == len(wpc)
        for st_, (key_, c_) in zip(WST, wpc.items()):
            ex = [q_copy(1)] + hi(2) if key_ == (0, 0) else []
            pre_ = hi(3) if key_ == (1, 0) else []
            sched[int(st_)] = sched.get(int(st_), []) + pre_ + [c_] + ex
    if SPL0:
        sched[-1] = lo0(0) + lo0(1)
    start(sched[-1])
    if MAN == 2:
        start(small[1:3])

    kvs = [kv0, kv1, kv2]
    r1[S:S + TM, XC:XC + D] = jnp.zeros((TM, D), bf16)
    wait(small if MAN == 1 else [small[0], small[3]])
    start(sched.get(-0.5, []))
    for j in range(8):
        zs[j] = 0
    zs[8] = 3
    zs[9] = 3 * PB
    zs[10] = TR2
    zs[12] = NR - 1
    zs[13] = 0
    zs[14] = TRA
    zs[11] = TR1
    dft_p[...] = _pack(dft_ref[...])
    for g in range(NG):
        tp = shk_ref[:, lanes(g)].astype(f32)
        for j in range(4):
            w[band(g) + OT, 8 * j:8 * j + 8, :] = _pack(jnp.broadcast_to(tp[j:j + 1], (8, 128)))

    def setup2():
        drow = dv_ref[...].astype(f32).reshape(1, D)
        for g in range(NG):
            par[g] = jnp.broadcast_to(drow[:, lanes(g)], (8, 128))
        eye = (jax.lax.broadcasted_iota(jnp.int32, (128, 128), 0)
               == jax.lax.broadcasted_iota(jnp.int32, (128, 128), 1))
        brow = bsp_ref[...].astype(f32).reshape(1, S)
        for t in range(S // 128):
            row = jnp.broadcast_to(brow[:, t * 128:(t + 1) * 128], (128, 128))
            col = jnp.sum(jnp.where(eye, row, 0.0), axis=1, keepdims=True)
            bcol[t * 128:(t + 1) * 128, :] = jnp.broadcast_to(col, (128, 128))

    if MAN == 1:
        setup2()

    hp = P // 2
    dep = {"rv": None, "out": [], "keep": None}

    def rel(x, on=None):
        if dep["rv"] is None or not (REL if on is None else on):
            return x
        return jnp.where(dep["keep"], x, dep["rv"])

    def done(x, lag=LAG):
        if dep["rv"] is not None:
            dep["out"].append((lag, x))

    def rel2(x):
        if dep["rv"] is None or not LREL:
            return x
        return jnp.concatenate(
            [jnp.concatenate([rel(x[r:r + 8, 0:128], 1), x[r:r + 8, 128:]], 1)
             for r in range(0, x.shape[0], 8)], 0)

    def done2(xp):
        for r in range(0, xp.shape[0], 8):
            for j in range(0, xp.shape[1] // 128, LDN):
                done(_f(xp[r:r + 8, j * 128:(j + 1) * 128]), LLAG)

    class Stage:
        def __init__(self, g, g0, h, base, base2=None):
            self.g, self.g0, self.h, self.base = g, g0, h, base
            self.base2 = base if base2 is None else base2
            self.early = isinstance(g, int) and g < MIG

        def uh(self, h):
            if h == 0:
                return w, self.base + band(self.g0)
            return uhh, (self.g0 % 2) * 48

        def yb(self, arr, t, pers):
            if pers:
                return self.base + band(self.g0) + OY + arr * 9 + (t - 7)
            return self.base + YT + (self.g0 % 2) * 27 + arr * 9 + (t + 1)

        def kv(self, b):
            if self.h == 0:
                return kvs[self.g % 3], (slice(b * hp, (b + 1) * hp), slice(None))
            return kvh, (self.g, slice(b * hp, (b + 1) * hp), slice(None))

        def dft(self, lo, n):
            return _unpack(dft_p[lo // 2:(lo + n) // 2, :])

    def h_mm(sa, b, h3):
        t0 = (sa.h * HB + b) * P
        hkb = r2[lanes(sa.g), 2 * D + t0:2 * D + t0 + P]
        dft = sa.dft
        if h3:
            t3 = jnp.concatenate(
                [_dot_nt(dft(P, 192), hkb), _dot_nt(dft(P + 192, 192), hkb)], 0)
            return jnp.concatenate([t3[P:2 * P], t3[2 * P:], t3[:P]], 0)
        c, d = _dot_nt(dft(2 * P, P), hkb), _dot_nt(dft(0, P), hkb)
        return jnp.concatenate([c, d - c, c + d], 0)

    def h_store(sa, b, hd, lo, n):
        ref, o = sa.uh(sa.h)
        ref[o + (3 + lo // P) * 8 + b, lo % P:lo % P + n, :] = _pack(hd[lo:lo + n])

    def kv_make(sa, b, nb):
        cols = lanes(sa.g)
        t0 = (sa.h * HB + b) * P
        n = nb * P
        taps = par[sa.g]
        if t0 == 0:
            kf_s[0:8, :] = jnp.zeros((8, 128), f32)
        elif b == 0:
            kf_s[0:8, :] = r2[t0 - 16:t0, cols].astype(f32)[8:16]
        l0 = b * P + 8
        kf_s[l0:l0 + n, :] = r2[t0:t0 + n, cols].astype(f32)
        ks = kf_s[l0:l0 + n, :] * taps[0:1]
        for j in range(1, 4):
            ks = ks + kf_s[l0 - j:l0 - j + n, :] * taps[j:j + 1]
        kv = _pack((ks * r2[t0:t0 + n, lanes(sa.g, D)].astype(f32)).astype(bf16))
        for j in range(nb):
            ref, idx = sa.kv(b + j)
            ref[idx] = kv[j * hp:(j + 1) * hp]

    def kv_fine(sa, b, q, nq):
        cols = lanes(sa.g)
        n = P // nq
        t0 = (sa.h * HB + b) * P + q * n
        l0 = b * P + q * n + 8
        if t0 == 0:
            kf_s[0:8, :] = jnp.zeros((8, 128), f32)
        elif l0 == 8:
            kf_s[0:8, :] = r2[t0 - 16:t0, cols].astype(f32)[8:16]
        kf_s[l0:l0 + n, :] = r2[t0:t0 + n, cols].astype(f32)
        tb = sa.base + band(sa.g0) + OT
        ks = None
        for j in range(4):
            tj = jnp.concatenate([rel(_f(w[tb, 8 * j:8 * j + 8, :]))] * (n // 8), 0)
            term = kf_s[l0 - j:l0 - j + n, :] * tj
            ks = term if ks is None else ks + term
        kv = _pack((ks * r2[t0:t0 + n, lanes(sa.g, D)].astype(f32)).astype(bf16))
        o = (b * P + q * n) // 2
        if sa.h:
            kvh[sa.g, o:o + n // 2, :] = kv
        else:
            kvs[sa.g % 3][o:o + n // 2, :] = kv
        for j in range(n // 16):
            done(_f(kv[8 * j:8 * j + 8]))

    def u_mm(sa, b, u3):
        ref, idx = sa.kv(b)
        kvb = _unpack(ref[idx])
        if u3:
            t3 = jnp.concatenate([_dot(sa.dft(0, 192), kvb), _dot(sa.dft(192, 192), kvb)], 0)
            return t3[2 * P:], t3[:P], t3[P:2 * P]
        return _dot(sa.dft(2 * P, P), kvb), _dot(sa.dft(0, P), kvb)

    def u_store(sa, b, u, rr):
        ref, o = sa.uh(sa.h)
        for a in range(2):
            ref[o + a * 8 + b, rr, :] = _pack(u[a][rr])
        ref[o + 16 + b, rr, :] = _pack(u[2][rr] if len(u) > 2 else u[0][rr] + u[1][rr])

    def c_prep(sb, sp, dup, bs=range(HB)):
        pers = sb.h == 1

        def ld(t, r0):
            s1, s3, s2 = (_f(w[sb.yb(a, t, pers), r0:r0 + 16, :]) for a in range(3))
            return s1 - s3, s1 + s2

        t0 = sb.h * HB + bs[0]
        prev = (ld(t0 - 1, sp * 16), ld(t0 - 1, hp + sp * 16)) if t0 else None
        for b in bs:
            t = sb.h * HB + b
            cur = (ld(t, sp * 16), ld(t, hp + sp * 16))
            (a0, c0), (a1, c1) = cur
            if prev is not None:
                a0, c0 = a0 - prev[0][1], c0 + prev[0][0]
                a1, c1 = a1 + prev[1][1], c1 - prev[1][0]
            prev = cur
            n = (sb.g0 % 2) * HB + b
            for j, v in enumerate((a0 + a1, c0 - c1, a0 - a1, c0 + c1)):
                v = _pack(v.astype(bf16))
                cbuf[n, j * 32 + sp * 8:j * 32 + sp * 8 + 8, :] = v
                done(_f(v))

    def c_mm(sc, b, tok):
        dft = sc.dft
        n = (sc.g0 % 2) * HB + b
        ye = tok(_dot(dft(4 * P, hp), _unpack(cbuf[n, 0:hp, :])))
        yo = _dot(dft(4 * P + hp, hp), _unpack(cbuf[n, hp:P, :]))
        ref, idx = sc.kv(b)
        kv, dd = ref[idx], par[sc.g][4:5]
        ys = [yy + dd * pltpu.unpack_elementwise(kv, index=j, packed_dtype=bf16, unpacked_dtype=f32)
              for j, yy in enumerate((ye, yo))]
        return _unpack(pltpu.pack_elementwise(ys, packed_dtype=bf16))

    def c_store(sc, b, y):
        t0 = (sc.h * HB + b) * P
        y_v[t0:t0 + P, lanes(sc.g)] = y

    def b_terms(sb, sl, arr, terms, init):
        r = slice(sl * 8, sl * 8 + 8)
        ha, ua = [(0, 2), (2, 1), (1, 0)][arr]
        out, hs, us, seen = {}, {}, {}, set()
        for t, uh_, b, hh_, d in terms:
            if t not in out and init(t):
                out[t] = _f(w[sb.yb(arr, t, True), r, :])
            if (hh_, d) not in hs:
                hr, ho = sb.uh(hh_)
                hs[hh_, d] = _f(hr[ho + (3 + ha) * 8 + d, r, :])
                if REL == 2:
                    hs[hh_, d] = rel(hs[hh_, d])
            if (uh_, b) not in us:
                ur, uo = sb.uh(uh_)
                us[uh_, b] = _f(ur[uo + ua * 8 + b, r, :])
            term = hs[hh_, d] * us[uh_, b]
            if t not in seen and REL == 1:
                term = rel(term)
            seen.add(t)
            out[t] = out[t] + term if t in out else term
        for t, val in out.items():
            done(val)
            if t <= 7:
                w[sb.yb(arr, t, False), r, :] = _pack(val)
            if t >= 7:
                w[sb.yb(arr, t, True), r, :] = _pack(val)

    def mk_terms(ts, sets, bs=range(8)):
        return [(t, uh_, b, hh_, t - 8 * uh_ - 8 * hh_ - b) for uh_, hh_ in sets for t in ts
                for b in bs if 0 <= t - 8 * uh_ - 8 * hh_ - b <= 7]

    def b_slice(sb, sl, kind, split=False):
        ab = [(1, 0), (0, 1)]
        if kind == "lo":
            groups = [(mk_terms(range(0, 8), [(0, 0)]), lambda t: False)]
        elif kind == "mi":
            groups = [(mk_terms(range(8, 15), [(0, 0)]), lambda t: False)]
        elif not split or BM == "pass":
            groups = [(mk_terms(range(8, 16), ab), lambda t: t < 15)]
        elif BM == "q4" and MI == 2 and not sb.early:
            ll = [(0, 0)]
            groups = [(mk_terms(range(8, 10), ll + ab), lambda t: False),
                      (mk_terms(range(10, 12), ll + ab), lambda t: False),
                      (mk_terms(range(12, 16), ab[:1], range(0, 4)), lambda t: False),
                      (mk_terms(range(12, 16), ab[1:], range(0, 4)), lambda t: True),
                      (mk_terms(range(12, 16), ll + ab, range(4, 8)), lambda t: True)]
        elif BM == "q4":
            groups = [(mk_terms(range(8, 12), ab), lambda t: True),
                      (mk_terms(range(12, 16), ab[:1], range(0, 4)), lambda t: t < 15),
                      (mk_terms(range(12, 16), ab[1:], range(0, 4)), lambda t: True),
                      (mk_terms(range(12, 16), ab, range(4, 8)), lambda t: True)]
        else:
            groups = [(mk_terms(range(8, 16), ab[:1]), lambda t: t < 15),
                      (mk_terms(range(8, 16), ab[1:]), lambda t: True)]
        fs = [lambda arr=arr, g=g: b_terms(sb, sl, arr, *g) for g in groups for arr in range(3)]
        if split:
            return fs
        for f in fs:
            f()

    def static_stage(s, zi):
        if s < 0 or s >= 2 * NG:
            return None
        if PREPIN == 0:
            return Stage(s % NG, s % NG, s // NG, 0)
        return Stage(s % NG, s % NG, s // NG, zab[min(zi, 1)], zab[0])

    def conv_pieces(sa, sb, sc, frac=1.0, h3=0, kq=KQ, psp=PSP, hg=HG, cof=COF):
        def hu(b, tok):
            hd = h_mm(sa, b, h3 & 1)
            u = u_mm(sa, b, h3 & 2)
            u = (tok(u[0]),) + tuple(u[1:])
            for a in range(3):
                h_store(sa, b, hd, a * P, P)
            u_store(sa, b, u, slice(0, P))

        def cc(b, tok):
            ys = [c_mm(sc, b + j, tok if j % (CG // 2) == 0 else lambda v: v) for j in range(CG)]
            for j in range(CG):
                c_store(sc, b + j, ys[j])

        mx, out = [], []
        d = 1.0 / (HB + 1.0)
        for b in range(HB):
            if sa:
                kvp = [lambda b=b, q=q: kv_fine(sa, b, q, kq) for q in range(kq)]
                mx.append((((b | (hg - 1)) + 1.2) * d, lambda tok, b=b: hu(b, tok), kvp))
                out += [((b + q / kq) * d, 200 / kq, f) for q, f in enumerate(kvp)]
            if sc and b % CG == 0:
                mx.append(((b / HB + cof) * frac, lambda tok, b=b: cc(b, tok), []))
        if sb:
            for sq in range(2 * HB):
                sl = (sq // 4) * 2 + sq % 2 + (sq % 4 // 2) * HB
                fs = b_slice(sb, sl, "hi", True) if sb.h else (
                    b_slice(sb, sl, "lo", True) + ([] if MI and not sb.early else b_slice(sb, sl, "mi", True)))
                fs = [((432.0 if MI < 2 or sb.early else CH if sb.h else CL) / len(fs), f) for f in fs]
                if sq % 4 == 3:
                    fs = fs + [(320 / psp, lambda sq=sq, bs=bs: c_prep(sb, sq // 4, True, bs))
                               for bs in _spread(list(range(HB)), psp)]
                for j, (c_, f) in enumerate(fs):
                    out.append(((sq + j / len(fs)) / (2.0 * HB), c_, f))
        return sorted(mx, key=lambda x: x[0]), sorted(out, key=lambda x: x[0])

    def scheduler(wts, pieces, rpt, lag, thin=TH1):
        cum = np.cumsum(wts) / np.sum(wts)
        slots = [[] for _ in wts]
        tot, run = sum(c_ for _, c_, _ in pieces), 0.0
        for _, c_, f in pieces:
            slots[min(int(np.searchsorted(cum, run / tot, side="right")), len(wts) - 1)].append(f)
            run += c_
        pend, cnt, ran = [], [0], []
        keep = jnp.full((8, 128), zs[5], jnp.int32) == 0

        def call(f):
            if not any(f is g for g in ran):
                ran.append(f)
                f()

        def need(fs):
            for f in fs:
                call(f)

        def tok(val):
            if not pieces:
                return val
            tiles = [val[r0:r0 + 8] for r0 in range(0, val.shape[0], 8)]
            for r0 in range(0, val.shape[0], rpt):
                due = [v for n, v in pend if n <= cnt[0]]
                pend[:] = [e for e in pend if e[0] > cnt[0]]
                for j, v in enumerate(due):
                    q = r0 // 8 + j % (rpt // 8)
                    tiles[q] = jnp.where(keep, tiles[q], v)
                dep["rv"], dep["out"], dep["keep"] = val[r0:r0 + 8], [], keep
                for f in slots[cnt[0]]:
                    call(f)
                pend.extend((cnt[0] + lag, v) for _, v in dep["out"][::-1][::thin])
                dep["rv"] = None
                cnt[0] += 1
            return jnp.concatenate(tiles, 0)

        return tok, need

    for s in range(NG + 2):
        if SPL0 and s == 0:
            wait(lo0(0))
        elif s == 1 and BPRE:
            pass
        elif not (NOW & 1 and s > 0 or NOW & 4):
            wait(grp_copies(s % NG, s // NG))
        start(sched.get(s, []))
        if MAN == 2 and s == 0:
            wait(small[1:3])
            setup2()
        if ONLY:
            continue
        mx, pieces = conv_pieces(static_stage(s, 0), static_stage(s - 1, 1),
                                 static_stage(s - 2, 2), h3=H3PRE, kq=KQ0, psp=PSP0, hg=1, cof=0.0)
        if s == 1 and BPRE:
            kvp = [f for e in mx for f in e[2]]
            bp = [e for e in pieces if not any(e[2] is f for f in kvp)]
            bp = bp[:int(len(bp) * BPRE)]
            for e in bp:
                e[2]()
            pieces = [e for e in pieces if not any(e is x for x in bp)]
            wait(grp_copies(1, 0))
        if SPL0 and s == 0:
            pieces = []
        tok, need = scheduler(sum([[1.0 if e[2] else WCC] * (P // RPT0) for e in mx], []), pieces, RPT0, LAG0, TH0)
        for j, (_, f, pre) in enumerate(mx):
            if SPL0 and s == 0 and j == SPL0:
                wait(lo0(1))
            need(pre)
            f(tok)

    npc = TM // PR

    def rows_of(i, r0=0, nr=TM):
        return pl.ds(pl.multiple_of(i * TM + r0, PR), nr)

    def a_layer_piece(r, i, iy, ps, stage_c):
        if not ps:
            return
        rr = rows_of(i, ps[0] * PR, len(ps) * PR)
        ry = rows_of(iy, ps[0] * PR, len(ps) * PR)
        x = r[rr, XC:XC + D].astype(f32)
        x = x + _ln(x) * y_v[ry, 0:D].astype(f32)
        r[rr, XC:XC + D] = x.astype(bf16)
        if stage_c is None:
            xnl[ps[0] * PR // 2:(ps[-1] + 1) * PR // 2, 0:D] = _pack(_ln(x).astype(bf16))
        else:
            r[rr, stage_c:stage_c + D] = _ln(x).astype(bf16)

    def norm_piece(r, i, ps):
        if not ps:
            return
        rr = rows_of(i, ps[0] * PR, len(ps) * PR)
        r[rr, FH:F] = _ln(r[rr, FH:F].astype(f32)).astype(bf16)

    nzh = FH // TN
    noc = D // TN

    def z_chunk(r, i, c, tn=TN, tok=lambda v: v, ks=1, r0=0, nr=TM):
        cs = slice(c * tn, (c + 1) * tn)
        kk = D // ks
        acc = None
        for k in range(ks):
            part = _dot(_unpack(xnl[r0 // 2:(r0 + nr) // 2, k * kk:(k + 1) * kk]),
                        win_v[k * kk:(k + 1) * kk, cs])
            if tn > 128 and ks > 1:
                part = jnp.concatenate([tok(part[:, 0:128]), part[:, 128:]], 1)
            else:
                part = tok(part)
            acc = part if acc is None else acc + part
        r[rows_of(i, r0, nr), cs] = _gelu(acc).astype(bf16)

    def g_chunk(r, i, c, side=None):
        cs = slice(c * TN, (c + 1) * TN)
        rr = rows_of(i)
        ks = KG if side else 1
        kk = S // ks
        gg = None
        for k in range(ks):
            if side:
                for f in side[c * ks + k]:
                    f()
            part = _dot(wsp_v[rr, k * kk:(k + 1) * kk],
                        r[k * kk:(k + 1) * kk, FH + c * TN:FH + (c + 1) * TN])
            gg = part if gg is None else gg + part
            if side:
                tk = gg[0:16, 0:128] if TKF else gg[TM - 16:TM, TN - 128:TN]
                r2[S:S + 16, 0:128] = tk.astype(bf16)
        bb = bcol[rr, :]
        gg = gg + jnp.concatenate([bb] * (TN // 128), axis=1)
        ml[:, cs] = _pack((r[rr, cs].astype(f32) * gg).astype(bf16))

    def o_chunk(src, dst, dst_c, i, c, r0=0, nr=TM):
        cs = slice(c * TN, (c + 1) * TN)
        rr = rows_of(i, r0, nr)
        o = _dot(_unpack(ml[r0 // 2:(r0 + nr) // 2, 0:FH]), wout_v[:, cs])
        x = src[rr, XC + c * TN:XC + (c + 1) * TN].astype(f32) + o
        dst[rr, dst_c + c * TN:dst_c + (c + 1) * TN] = x.astype(bf16)

    parts_z = _spread(list(range(npc)), nzh)
    parts_o = _spread(list(range(npc)), noc)

    def finish(pending):
        wait(pending)
        out_copy(NR - 1).start()
        out_copy(NR - 1).wait()

    late = sum([hi(g) for g in range(4, NG)], []) + [q_copy(i) for i in range(2, NR)]
    if not LATE:
        start(late)
    if not NOW & 2:
        q_copy(0).wait()
    for ps in (_spread(list(range(npc // 2)), 4) if ZRS else parts_z):
        a_layer_piece(r1, 0, 0, ps, 0)
    if not NOW & 2:
        wait(win_copy if W1 == 0 else win_copy[:1])
    if STOP == 1:
        finish([c for g in range(2, NG) for c in grp_copies(g, 1)] + [q_copy(i) for i in range(1, NR)])
        return
    if not LATE:
        start([wsp_copy, wout_copy])

    def ln_pieces(fn, lo=0.0, hi=1.0, n=LNP, sub=None):
        d = (hi - lo) / n
        return [(lo + j * d, lambda ps=ps: fn(ps))
                for j, ps in enumerate(_spread(sub or list(range(npc)), n))]

    def p1_half(i, hh, lnp, conv=((), ()), hook=None, zrs=0):
        mx, pieces = conv
        if NOLN & (1 << hh) and pieces:
            lnp = []
        tn = TN1 if pieces else TNC
        nz1 = FH // tn
        ks = 2 * tn // 128
        rpt = TM // TPS
        grp = [[e for e in mx if min(int(e[0] * nz1 + 1e-6), nz1 - 1) == c] for c in range(nz1)]
        wts = []
        for c in range(nz1):
            for e in grp[c]:
                wts += [WC if e[2] else WC * WCC] * (P // rpt)
            wts += [1.0] * (TPS * (ks - 1)) + [W0] * TPS
        tok, need = scheduler(wts, pieces, rpt, LAG)
        for c in range(nz1):
            if hook and c and (hh, c * tn // 128) in wpc:
                hook(wpc[hh, c * tn // 128].wait)
            for p_, f in lnp:
                if min(int(p_ * nz1 + 1e-6), nz1 - 1) == c:
                    f()
            for _, f, pre in grp[c]:
                need(pre)
                f(tok)
            if c < zrs:
                hm = TM // 2
                a0 = _spread(list(range(npc // 2, npc)), ZNP)
                for k in (2 * c, 2 * c + 1):
                    if k < ZNP:
                        a_layer_piece(r1, i, i, a0[k], 0)
                    if k == zrs:
                        xnl[hm // 2:hm, 0:D] = _pack(r1[rows_of(i, hm, hm), 0:D])
                    z_chunk(r1, i, k % zrs + nz1, tn, tok, ks, k // zrs * hm, hm)
                continue
            z_chunk(r1, i, c + (nz1 if hh == 0 else 0), tn, tok, ks if pieces else 1)

    def p1a_body(i, carry, first=None):
        def once(f):
            if first is None:
                pl.when(i == 0)(f)
            elif first:
                f()

        hk0 = hk1 = once if first is not False else None
        i0 = i
        if TRA:
            i = jnp.minimum(i, 2)

            @pl.when(i0 < 3)
            def _():
                q_copy(i + 1).wait()
                wait(grp_copies(2 * i + 2, 1))
        elif not NOW & 2:
            q_copy(i + 1).wait()
            wait(grp_copies(2 * i + 2, 1))
        if W1 < 2:
            wait(grp_copies(2 * i + 3, 1))
        base = i * PB

        def st(g0):
            sg = Stage(2 * i + g0, g0, 1, base)
            sg.early = bool(first) and g0 < MIG
            return sg

        zr = ZRS if first else 0
        nx = TM // 2 if zr else TM
        xnl[0:nx // 2, 0:D] = _pack(r1[rows_of(i, 0, nx), 0:D])
        al = lambda ps: a_layer_piece(r1, i + 1, i + 1, ps, 0)
        h0, h1 = list(range(npc // 2)), list(range(npc // 2, npc))
        p1_half(i, 0, ln_pieces(al, 0.35 if zr else 0.0, n=LNH, sub=h0),
                conv_pieces(st(2), st(1), st(0)), hk0, zr)
        if TRA:
            @pl.when(i0 < 3)
            def _():
                wait(grp_copies(2 * i + 3, 1))
        elif W1 >= 2 and not NOW & 2:
            wait(grp_copies(2 * i + 3, 1))
        if W1 == 2:
            def mid():
                win_copy[1].wait()
                start(late)

            once(mid)
        p1_half(i, 1, [ln_pieces(lambda ps: norm_piece(r1, i, ps), n=LNA), [],
                       ln_pieces(al, n=LNH, sub=h1)][DEFN],
                conv_pieces(st(3), st(2), st(1)), hk1)
        return carry

    if ONLY != 'p1c':
        if WQ == 2:
            p1a_body(zs[13], 0, True)
            jax.lax.fori_loop(1, 3, lambda i, cr: p1a_body(i, cr, False), 0)
        else:
            jax.lax.fori_loop(0, zs[14] if TRA else 3, p1a_body, 0)
    else:
        wait([q_copy(i) for i in range(1, 4)] + [c for g in range(2, NG) for c in grp_copies(g, 1)])

    if W1 in (1, 3):
        win_copy[1].wait()
    if LATE:
        start([wsp_copy, wout_copy])
    if NOW & 2:
        wait(win_copy + [q_copy(i) for i in range(4)] + sum([hi(g) for g in range(2, NG)], []))
    if NOW & 5:
        wait(sum([list(grp_copies(s % NG, s // NG)) for s in range(0 if NOW & 4 else 1, NG + 2)], []))
    wait([q_copy(i) for i in range(4, NR)])
    if ONLY == 'p1a':
        finish([wsp_copy, wout_copy])
        return
    i3 = zs[8]
    xnl[:, 0:D] = _pack(r1[rows_of(i3), 0:D])
    if DYNB:
        b3 = zs[9]
        s14, s15 = Stage(2 * i3, 0, 1, b3), Stage(2 * i3 + 1, 1, 1, b3)
    else:
        s14, s15 = static_stage(14, 0), static_stage(15, 0)
    p1_half(i3, 0, [], conv_pieces(None, s15, s14))
    p1_half(i3, 1, ([] if DEFN else ln_pieces(lambda ps: norm_piece(r1, i3, ps), 0.0, 0.5, 4))
            + ln_pieces(lambda ps: a_layer_piece(r1, i3 + 1, i3 + 1, ps, 0), 0.45, 1.0, 4),
            conv_pieces(None, None, s15, 0.4))

    def p1c_body(i, carry):
        iy = jnp.minimum(i + 1, NR - 1)
        xnl[:, 0:D] = _pack(r1[rows_of(i), 0:D])
        n4 = lambda ps: norm_piece(r1, i - 4, ps)
        p1_half(i, 0, ln_pieces(lambda ps: a_layer_piece(r1, i + 1, iy, ps, 0))
                + (ln_pieces(n4, n=DNS // 2, sub=list(range(DNS))) if DNS else []))
        p1_half(i, 1, ln_pieces(lambda ps: norm_piece(r1, i, ps))
                + ln_pieces(n4, n=min(7, (npc - DNS) // 2), sub=list(range(DNS, npc))))
        return carry

    if U1 == 1:
        jax.lax.fori_loop(4, zs[11] if TR1 else NR, p1c_body, 0)
    else:
        jax.lax.fori_loop(2, 4, lambda j, cr: p1c_body(2 * j + 1, p1c_body(2 * j, cr)), 0)

    wsp_copy.wait()
    wout_copy.wait()
    if STOP == 2:
        finish([])
        return

    last = NR - 1
    parts_a = _spread(list(range(npc)), NA2) + [[]] * (nzh - NA2)

    def g_side(i, ia, inorm):
        pp = [list(range(j, j + PG)) for j in range(0, npc, PG)]
        base = ia * TM

        def rws(ps, off=0):
            return pl.ds(pl.multiple_of(base + (off + ps[0] * PR), PR), len(ps) * PR)

        def cp(ps):
            xnl[ps[0] * PR // 2:(ps[-1] + 1) * PR // 2, 0:D] = _pack(r2[rws(ps), FH:FH + D])

        def a2a(ps):
            rr = rws(ps)
            x = r2[rr, XC:XC + D].astype(f32)
            r2[rr, XC:XC + D] = (x + _ln(x) * y_v[rr, 0:D].astype(f32)).astype(bf16)

        def a2b(ps):
            rr = rws(ps)
            r2[rr, FH:FH + D] = _ln(r2[rr, XC:XC + D].astype(f32)).astype(bf16)

        def nrm(ps):
            rr = rws(ps, -TM)
            r2[rr, FH:F] = _ln(r2[rr, FH:F].astype(f32)).astype(bf16)

        nw = nzh * KG
        seq = []
        for j, ps in enumerate(pp):
            seq.append([lambda ps=ps: a2a(ps)])
            if j:
                seq[-1].insert(0, lambda ps=pp[j - 1]: cp(ps))
            if inorm is not None:
                seq.append([lambda ps=ps: nrm(ps)])
            seq.append([lambda ps=ps: a2b(ps)])
        seq.append([lambda: cp(pp[-1])])
        side = [sum(x, []) for x in _spread(seq, nw - NA2)] + [[]] * NA2
        for c in range(nzh):
            g_chunk(r1, i, c, side)

    def p2r_body(i, carry):
        for c in range(nzh):
            z_chunk(r2, i - 1, nzh + c)
        for c in range(noc):
            o_chunk(r1, r2, XC, i, c)
        for c in range(nzh):
            z_chunk(r2, i - 1, c)
        g_side(i + 1, i, i - 1)
        return carry

    if ROT:
        for c in range(nzh):
            g_chunk(r1, 0, c)
        for c in range(noc):
            o_chunk(r1, r2, XC, 0, c)
        g_side(1, zs[13], None)
        jax.lax.fori_loop(1, NR - 1, p2r_body, 0)
        i7 = zs[12]
        for c in range(nzh):
            z_chunk(r2, i7 - 1, nzh + c)
        for c in range(noc):
            if EPI & 1:
                norm_piece(r2, i7 - 1, parts_o[c])
            o_chunk(r1, r2, XC, i7, c)
        for c in range(nzh):
            a_layer_piece(r2, i7, i7, parts_z[c], FH)
            z_chunk(r2, i7 - 1, c)
        xnl[:, 0:D] = _pack(r2[rows_of(last), FH:FH + D])
        for c in range(nzh):
            if not EPI & 1:
                norm_piece(r2, i7 - 1, parts_z[c])
            z_chunk(r2, i7 if EPI & 4 else last, nzh + c)
        for c in range(nzh):
            norm_piece(r2, i7 if EPI & 2 else last, parts_z[c])
            z_chunk(r2, i7 if EPI & 4 else last, c)
    else:
        for c in range(nzh):
            g_chunk(r1, 0, c)
        if ORS:
            np1 = ORS // PR
            for c in range(noc):
                o_chunk(r1, r2, XC, 0, c, 0, ORS)
            for c, ps in enumerate(_spread(list(range(np1)), noc)):
                a_layer_piece(r2, zs[13], zs[13], ps, FH)
                o_chunk(r1, r2, XC, 0, c, ORS, TM - ORS)
            for ps in _spread(list(range(np1, npc)), 4):
                a_layer_piece(r2, 0, 0, ps, FH)
        else:
            for c in range(noc):
                o_chunk(r1, r2, XC, 0, c)
            for ps in parts_z:
                a_layer_piece(r2, 0, 0, ps, FH)

        def p2_body(i, carry):
            xnl[:, 0:D] = _pack(r2[rows_of(i - 1), FH:FH + D])
            for c in range(nzh):
                g_chunk(r1, i, c)
            if P2O:
                for c in range(noc):
                    o_chunk(r1, r2, XC, i, c)
                for c in range(nzh):
                    a_layer_piece(r2, i, i, parts_z[c], FH)
                    z_chunk(r2, i - 1, nzh + c)
                for c in range(nzh):
                    norm_piece(r2, i - 1, parts_z[c])
                    z_chunk(r2, i - 1, c)
                return carry
            for c in range(nzh):
                z_chunk(r2, i - 1, nzh + c)
            for c in range(noc):
                norm_piece(r2, i - 1, parts_o[c])
                o_chunk(r1, r2, XC, i, c)
            for c in range(nzh):
                a_layer_piece(r2, i, i, parts_z[c], FH)
                z_chunk(r2, i - 1, c)
            return carry

        if U2 == 1:
            jax.lax.fori_loop(1, zs[10] if TR2 else NR, p2_body, 0)
        else:
            jax.lax.fori_loop(0, 3, lambda j, cr: p2_body(2 * j + 2, p2_body(2 * j + 1, cr)), 0)
            p2_body(zs[12], 0)

        last = NR - 1
        xnl[:, 0:D] = _pack(r2[rows_of(last), FH:FH + D])
        for c in range(nzh):
            z_chunk(r2, last, nzh + c)
        for c in range(nzh):
            norm_piece(r2, zs[12] if EPI & 2 else last, parts_z[c])
            z_chunk(r2, last, c)

    for c in range(nzh):
        g_chunk(r2, 0, c)

    def p3_body(i, carry):
        for c in range(noc):
            o_chunk(r2, y_v, 0, i - 1, c)
        out_copy(i - 1).start()
        for c in range(nzh):
            g_chunk(r2, i, c)
        return carry

    if U3 == 1:
        jax.lax.fori_loop(1, NR, p3_body, 0)
    elif U3 == 2:
        jax.lax.fori_loop(0, 3, lambda j, cr: p3_body(2 * j + 2, p3_body(2 * j + 1, cr)), 0)
        p3_body(NR - 1, 0)
    else:
        for i in range(1, NR):
            p3_body(i, 0)
    def out_last(c):
        cs = slice(c * TN, (c + 1) * TN)
        return pltpu.make_async_copy(y_v.at[blk(last), cs], out_hbm.at[0, blk(last), cs],
                                     sem_o.at[NR + c])

    for c in range(noc):
        o_chunk(r2, y_v, 0, NR - 1, c)
        if OSP:
            out_last(c).start()
    if not OSP:
        out_copy(NR - 1).start()
    for i in range(NR - OSP):
        out_copy(i).wait()
    if OSP:
        wait([out_last(c) for c in range(noc)])


@jax.jit
def pallas_interleave_layers__ssm_conv_h3__mixer_gmlp__prompt_kernel(
    A_q, A_k, A_v, A_shift_k, A_ssm_k, A_ssm_D, B_x, B_w_in, B_w_sp, B_b_sp, B_w_out,
):
    del B_x
    anyspec = pl.BlockSpec(memory_space=pl.ANY)
    vmem = pl.BlockSpec(memory_space=pltpu.VMEM)
    return pl.pallas_call(
        _kernel,
        grid=(1,),
        in_specs=[anyspec] * 11,
        out_specs=anyspec,
        out_shape=jax.ShapeDtypeStruct((1, S, D), bf16),
        scratch_shapes=[
            pltpu.VMEM((D, F + PS3), bf16),
            pltpu.VMEM((S, S + PS1), bf16),
            pltpu.VMEM((FH, D + PS2), bf16),
            pltpu.VMEM((S, D + PS5), bf16),
            pltpu.VMEM((S + TM, RW), bf16),
            pltpu.VMEM((S + 16, RW), bf16),
            pltpu.VMEM((TM // 2, D + PS4), u32),
            pltpu.VMEM((TM // 2, FH + PS6), u32),
            pltpu.VMEM((NTW, P + PADW, 128), u32),
            pltpu.VMEM((96, P + PADW, 128), u32),
            pltpu.VMEM((HS // 2, 128), u32),
            pltpu.VMEM((HS // 2, 128), u32),
            pltpu.VMEM((HS // 2, 128), u32),
            pltpu.VMEM((NG, HS // 2, 128), u32),
            pltpu.VMEM((2 * HB, P + PADW, 128), u32),
            pltpu.VMEM((HS + 8, 128), f32),
            pltpu.VMEM((5 * P // 2, 128), u32),
            pltpu.VMEM((S, 128), f32),
            pltpu.VMEM((NG, 8, 128), f32),
            pltpu.SMEM((16,), jnp.int32),
            pltpu.VMEM((4, D), bf16),
            pltpu.VMEM((D,), bf16),
            pltpu.VMEM((S,), bf16),
            pltpu.VMEM((5 * P, 128), bf16),
            pltpu.SemaphoreType.DMA((2 * NG,)),
            pltpu.SemaphoreType.DMA((2 * NG,)),
            pltpu.SemaphoreType.DMA((2 * NG,)),
            pltpu.SemaphoreType.DMA((16,)),
            pltpu.SemaphoreType.DMA((NR,)),
            pltpu.SemaphoreType.DMA((NR + 4,)),
            pltpu.SemaphoreType.DMA((7,)),
        ],
        compiler_params=pltpu.CompilerParams(
            dimension_semantics=("arbitrary",),
            vmem_limit_bytes=124 * 1024 * 1024,
        ),
    )(A_q, A_k, A_v, A_shift_k.T, A_ssm_k, A_ssm_D, B_w_in, B_w_sp, B_b_sp, B_w_out,
      _dft_constants())
```

```python
import numpy as np
import jax
import jax.numpy as jnp
import jax.experimental.pallas as pl
import jax.experimental.pallas.tpu as pltpu
S = 2048
D = 1024
F = 3584
FH = F // 2
P = 128
NB = S // P
HB = NB // 2
HS = S // 2
NG = D // 128
TM = 256
NR = S // TM
TN = 256
PR = 16
XC = F
RW = F + D
EPS = 1e-05
MIG = 1
CG = 4
ORS = 128
TPS = 8
W0 = 0.8
LNP = 7
TN1 = 128
PSP = 3
KQ = 4
WC = 1.0
LAG = 2
KQ0 = 2
PSP0 = 2
RPT0 = 16
LAG0 = 3
TNC = 256
BPRE = 0.15
WB0 = '0 7 14'.split()
WB1 = '0 7 14'.split()
DS = '0 0 1 2 2 3 4 5 5 6 7 7 8 9 9 9'.split()
A4L = 0.143
A4N = 6
A4F = 0.1
CH = 500
CL = 250
PADW = 8
PS2 = 128
LNH = 5
OSP = 1
BS = 76
OY = 48
OT = 75
PB = 2 * BS
YT = 4 * PB
TK = YT + 54
NTW = TK

def band(n):
    return n * BS
f32 = jnp.float32
bf16 = jnp.bfloat16
u32 = jnp.uint32

def _dft_constants():
    n = np.arange(P)
    k = np.concatenate([np.arange(0, P, 2), P - 1 - np.arange(0, P, 2)])
    ang = 2.0 * np.pi * np.outer(2 * k + 1, n) / (4 * P)
    fre, fim = (np.cos(ang), -np.sin(ang))
    gi = np.concatenate([fre[:P // 2].T, fim[:P // 2].T], 1) / P
    g = np.concatenate([gi[0::2], gi[1::2]], 0)
    return jnp.asarray(np.concatenate([fim, fre, g], 0), dtype=bf16)

def _ln(x):
    m = jnp.mean(x, axis=-1, keepdims=True)
    xc = x - m
    v = jnp.mean(xc * xc, axis=-1, keepdims=True)
    return xc * jax.lax.rsqrt(v + EPS)

def _gelu(z):
    c = 0.7978845608028654
    u = z * (c + c * 0.044715 * (z * z))
    h = 0.5 * z
    return h + h * jnp.tanh(u)

def _dot(a, b):
    return jnp.dot(a, b, preferred_element_type=f32)

def _spread(work, n):
    return [work[j * len(work) // n:(j + 1) * len(work) // n] for j in range(n)]

def _dot_nt(a, b):
    return jax.lax.dot_general(a, b, (((1,), (1,)), ((), ())), preferred_element_type=f32)

def _pack(x):
    return pltpu.bitcast(x, u32)

def _unpack(x):
    return pltpu.bitcast(x, bf16)

def _f(x):
    return pltpu.bitcast(x, f32)

def _kernel(q_hbm, k_hbm, v_hbm, shk_hbm, hk_hbm, dv_hbm, win_hbm, wsp_hbm, bsp_hbm, wout_hbm, dft_hbm, out_hbm, win_v, wsp_v, wout_v, y_v, r1, r2, xnl, ml, w, uhh, kv0, kv1, kv2, kvh, cbuf, kf_s, dft_p, bcol, par, zs, shk_ref, dv_ref, bsp_ref, dft_ref, sem_k, sem_v, sem_h, sem_w, sem_q, sem_o, sem_s):
    small = [pltpu.make_async_copy(a, b, sem_s.at[j]) for j, (a, b) in enumerate([(shk_hbm, shk_ref), (dv_hbm, dv_ref), (bsp_hbm, bsp_ref), (dft_hbm, dft_ref)])]
    for c in [small[0], small[3]]:
        c.start()

    def lanes(g, off=0):
        if isinstance(g, int):
            return slice(off + g * 128, off + (g + 1) * 128)
        return pl.ds(pl.multiple_of(off + g * 128, 128), 128)

    def grp_copies(g, h):
        cols, rows = (lanes(g), slice(h * HS, (h + 1) * HS))
        s = h * NG + g
        hrows = slice(2 * D + h * HS, 2 * D + (h + 1) * HS)
        return (pltpu.make_async_copy(hk_hbm.at[cols, rows], r2.at[cols, hrows], sem_h.at[s]), pltpu.make_async_copy(k_hbm.at[0, rows, cols], r2.at[rows, cols], sem_k.at[s]), pltpu.make_async_copy(v_hbm.at[0, rows, cols], r2.at[rows, lanes(g, D)], sem_v.at[s]))

    def blk(i):
        if isinstance(i, int):
            return slice(i * TM, (i + 1) * TM)
        return pl.ds(pl.multiple_of(i * TM, TM), TM)

    def q_copy(i):
        return pltpu.make_async_copy(q_hbm.at[0, blk(i), :], r1.at[blk(i), XC:XC + D], sem_q.at[i])
    wb = [[int(x) for x in WB0], [int(x) for x in WB1]]
    wpc = {}
    for hh_ in range(2):
        for a_, b_ in zip(wb[hh_][:-1], wb[hh_][1:]):
            cs_ = slice((1 - hh_) * FH + a_ * 128, (1 - hh_) * FH + b_ * 128)
            wpc[hh_, a_] = pltpu.make_async_copy(win_hbm.at[:, cs_], win_v.at[:, cs_], sem_w.at[4 + len(wpc)])
    win_copy = [wpc[0, 0], wpc[1, 0]]
    wsp_copy = pltpu.make_async_copy(wsp_hbm, wsp_v.at[:, 0:S], sem_w.at[2])
    wout_copy = pltpu.make_async_copy(wout_hbm, wout_v.at[:, 0:D], sem_w.at[3])

    def out_copy(i):
        return pltpu.make_async_copy(y_v.at[blk(i), 0:D], out_hbm.at[0, blk(i), :], sem_o.at[i])

    def start(cs):
        for c in cs:
            c.start()

    def wait(cs):
        for c in cs:
            c.wait()
    lo = lambda g: list(grp_copies(g, 0))
    hi = lambda g: list(grp_copies(g, 1))
    wl = list(wpc.values())
    need = [lo(g) for g in range(2, NG)] + [hi(0), hi(1), [q_copy(0)], wl[0:1], [q_copy(1)], hi(2), wl[1:2], hi(3), wl[2:3], wl[3:4]]
    sched = {-1: lo(0), -0.5: lo(1)}
    for st_, cs_ in zip(DS, need):
        sched[int(st_)] = sched.get(int(st_), []) + cs_
    start(sched[-1])
    start(small[1:3])
    kvs = [kv0, kv1, kv2]
    r1[S:S + TM, XC:XC + D] = jnp.zeros((TM, D), bf16)
    wait([small[0], small[3]])
    start(sched.get(-0.5, []))
    for j in range(8):
        zs[j] = 0
    zs[8] = 3
    zs[9] = 3 * PB
    zs[12] = NR - 1
    zs[13] = 0
    dft_p[...] = _pack(dft_ref[...])
    for g in range(NG):
        tp = shk_ref[:, lanes(g)].astype(f32)
        for j in range(4):
            w[band(g) + OT, 8 * j:8 * j + 8, :] = _pack(jnp.broadcast_to(tp[j:j + 1], (8, 128)))

    def setup2():
        drow = dv_ref[...].astype(f32).reshape(1, D)
        for g in range(NG):
            par[g] = jnp.broadcast_to(drow[:, lanes(g)], (8, 128))
        eye = jax.lax.broadcasted_iota(jnp.int32, (128, 128), 0) == jax.lax.broadcasted_iota(jnp.int32, (128, 128), 1)
        brow = bsp_ref[...].astype(f32).reshape(1, S)
        for t in range(S // 128):
            row = jnp.broadcast_to(brow[:, t * 128:(t + 1) * 128], (128, 128))
            col = jnp.sum(jnp.where(eye, row, 0.0), axis=1, keepdims=True)
            bcol[t * 128:(t + 1) * 128, :] = jnp.broadcast_to(col, (128, 128))

    hp = P // 2
    dep = {'rv': None, 'out': []}

    def done(x, lag=LAG):
        if dep['rv'] is not None:
            dep['out'].append((lag, x))

    class Stage:
        def __init__(self, g, g0, h, base, base2=None):
            self.g, self.g0, self.h, self.base = (g, g0, h, base)
            self.base2 = base if base2 is None else base2
            self.early = isinstance(g, int) and g < MIG

        def uh(self, h):
            if h == 0:
                return (w, self.base + band(self.g0))
            return (uhh, self.g0 % 2 * 48)

        def yb(self, arr, t, pers):
            if pers:
                return self.base + band(self.g0) + OY + arr * 9 + (t - 7)
            return self.base + YT + self.g0 % 2 * 27 + arr * 9 + (t + 1)

        def kv(self, b):
            if self.h == 0:
                return (kvs[self.g % 3], (slice(b * hp, (b + 1) * hp), slice(None)))
            return (kvh, (self.g, slice(b * hp, (b + 1) * hp), slice(None)))

        def dft(self, lo, n):
            return _unpack(dft_p[lo // 2:(lo + n) // 2, :])

    def h_mm(sa, b):
        t0 = (sa.h * HB + b) * P
        hkb = r2[lanes(sa.g), 2 * D + t0:2 * D + t0 + P]
        dft = sa.dft
        c, d = (_dot_nt(dft(P, P), hkb), _dot_nt(dft(0, P), hkb))
        return jnp.concatenate([c, d - c, c + d], 0)

    def h_store(sa, b, hd, lo, n):
        ref, o = sa.uh(sa.h)
        ref[o + (3 + lo // P) * 8 + b, lo % P:lo % P + n, :] = _pack(hd[lo:lo + n])

    def kv_fine(sa, b, q, nq):
        cols = lanes(sa.g)
        n = P // nq
        t0 = (sa.h * HB + b) * P + q * n
        l0 = b * P + q * n + 8
        if t0 == 0:
            kf_s[0:8, :] = jnp.zeros((8, 128), f32)
        elif l0 == 8:
            kf_s[0:8, :] = r2[t0 - 16:t0, cols].astype(f32)[8:16]
        kf_s[l0:l0 + n, :] = r2[t0:t0 + n, cols].astype(f32)
        tb = sa.base + band(sa.g0) + OT
        ks = None
        for j in range(4):
            tj = jnp.concatenate([_f(w[tb, 8 * j:8 * j + 8, :])] * (n // 8), 0)
            term = kf_s[l0 - j:l0 - j + n, :] * tj
            ks = term if ks is None else ks + term
        kv = _pack((ks * r2[t0:t0 + n, lanes(sa.g, D)].astype(f32)).astype(bf16))
        o = (b * P + q * n) // 2
        if sa.h:
            kvh[sa.g, o:o + n // 2, :] = kv
        else:
            kvs[sa.g % 3][o:o + n // 2, :] = kv
        for j in range(n // 16):
            done(_f(kv[8 * j:8 * j + 8]))

    def u_mm(sa, b):
        ref, idx = sa.kv(b)
        kvb = _unpack(ref[idx])
        return (_dot(sa.dft(P, P), kvb), _dot(sa.dft(0, P), kvb))

    def u_store(sa, b, u, rr):
        ref, o = sa.uh(sa.h)
        for a in range(2):
            ref[o + a * 8 + b, rr, :] = _pack(u[a][rr])
        ref[o + 16 + b, rr, :] = _pack(u[0][rr] + u[1][rr])

    def c_prep(sb, sp, dup, bs=range(HB)):
        pers = sb.h == 1

        def ld(t, r0):
            s1, s3, s2 = (_f(w[sb.yb(a, t, pers), r0:r0 + 16, :]) for a in range(3))
            return (s1 - s3, s1 + s2)
        t0 = sb.h * HB + bs[0]
        prev = (ld(t0 - 1, sp * 16), ld(t0 - 1, hp + sp * 16)) if t0 else None
        for b in bs:
            t = sb.h * HB + b
            cur = (ld(t, sp * 16), ld(t, hp + sp * 16))
            (a0, c0), (a1, c1) = cur
            if prev is not None:
                a0, c0 = (a0 - prev[0][1], c0 + prev[0][0])
                a1, c1 = (a1 + prev[1][1], c1 - prev[1][0])
            prev = cur
            n = sb.g0 % 2 * HB + b
            for j, v in enumerate((a0 + a1, c0 - c1, a0 - a1, c0 + c1)):
                v = _pack(v.astype(bf16))
                cbuf[n, j * 32 + sp * 8:j * 32 + sp * 8 + 8, :] = v
                done(_f(v))

    def c_mm(sc, b, tok):
        dft = sc.dft
        n = sc.g0 % 2 * HB + b
        ye = tok(_dot(dft(2 * P, hp), _unpack(cbuf[n, 0:hp, :])))
        yo = _dot(dft(2 * P + hp, hp), _unpack(cbuf[n, hp:P, :]))
        ref, idx = sc.kv(b)
        kv, dd = (ref[idx], par[sc.g][4:5])
        ys = [yy + dd * pltpu.unpack_elementwise(kv, index=j, packed_dtype=bf16, unpacked_dtype=f32) for j, yy in enumerate((ye, yo))]
        return _unpack(pltpu.pack_elementwise(ys, packed_dtype=bf16))

    def c_store(sc, b, y):
        t0 = (sc.h * HB + b) * P
        y_v[t0:t0 + P, lanes(sc.g)] = y

    def b_terms(sb, sl, arr, terms, init):
        r = slice(sl * 8, sl * 8 + 8)
        ha, ua = [(0, 2), (2, 1), (1, 0)][arr]
        out, hs, us = ({}, {}, {})
        for t, uh_, b, hh_, d in terms:
            if t not in out and init(t):
                out[t] = _f(w[sb.yb(arr, t, True), r, :])
            if (hh_, d) not in hs:
                hr, ho = sb.uh(hh_)
                hs[hh_, d] = _f(hr[ho + (3 + ha) * 8 + d, r, :])
            if (uh_, b) not in us:
                ur, uo = sb.uh(uh_)
                us[uh_, b] = _f(ur[uo + ua * 8 + b, r, :])
            term = hs[hh_, d] * us[uh_, b]
            out[t] = out[t] + term if t in out else term
        for t, val in out.items():
            done(val)
            if t <= 7:
                w[sb.yb(arr, t, False), r, :] = _pack(val)
            if t >= 7:
                w[sb.yb(arr, t, True), r, :] = _pack(val)

    def mk_terms(ts, sets, bs=range(8)):
        return [(t, uh_, b, hh_, t - 8 * uh_ - 8 * hh_ - b) for uh_, hh_ in sets for t in ts for b in bs if 0 <= t - 8 * uh_ - 8 * hh_ - b <= 7]

    def b_slice(sb, sl, kind, split=False):
        ab = [(1, 0), (0, 1)]
        if kind == 'lo':
            groups = [(mk_terms(range(0, 8), [(0, 0)]), lambda t: False)]
        elif kind == 'mi':
            groups = [(mk_terms(range(8, 15), [(0, 0)]), lambda t: False)]
        elif not split:
            groups = [(mk_terms(range(8, 16), ab), lambda t: t < 15)]
        elif not sb.early:
            ll = [(0, 0)]
            groups = [(mk_terms(range(8, 10), ll + ab), lambda t: False), (mk_terms(range(10, 12), ll + ab), lambda t: False), (mk_terms(range(12, 16), ab[:1], range(0, 4)), lambda t: False), (mk_terms(range(12, 16), ab[1:], range(0, 4)), lambda t: True), (mk_terms(range(12, 16), ll + ab, range(4, 8)), lambda t: True)]
        else:
            groups = [(mk_terms(range(8, 12), ab), lambda t: True), (mk_terms(range(12, 16), ab[:1], range(0, 4)), lambda t: t < 15), (mk_terms(range(12, 16), ab[1:], range(0, 4)), lambda t: True), (mk_terms(range(12, 16), ab, range(4, 8)), lambda t: True)]
        fs = [lambda arr=arr, g=g: b_terms(sb, sl, arr, *g) for g in groups for arr in range(3)]
        if split:
            return fs
        for f in fs:
            f()

    def static_stage(s, zi):
        if s < 0 or s >= 2 * NG:
            return None
        return Stage(s % NG, s % NG, s // NG, 0)

    def conv_pieces(sa, sb, sc, frac=1.0, kq=KQ, psp=PSP):
        def hu(b, tok):
            hd = h_mm(sa, b)
            u = u_mm(sa, b)
            u = (tok(u[0]),) + tuple(u[1:])
            for a in range(3):
                h_store(sa, b, hd, a * P, P)
            u_store(sa, b, u, slice(0, P))

        def cc(b, tok):
            ys = [c_mm(sc, b + j, tok if j % (CG // 2) == 0 else lambda v: v) for j in range(CG)]
            for j in range(CG):
                c_store(sc, b + j, ys[j])
        mx, out = ([], [])
        d = 1.0 / (HB + 1.0)
        for b in range(HB):
            if sa:
                kvp = [lambda b=b, q=q: kv_fine(sa, b, q, kq) for q in range(kq)]
                mx.append(((b + 1.2) * d, lambda tok, b=b: hu(b, tok), kvp))
                out += [((b + q / kq) * d, 200 / kq, f) for q, f in enumerate(kvp)]
            if sc and b % CG == 0:
                mx.append((b / HB * frac, lambda tok, b=b: cc(b, tok), []))
        if sb:
            for sq in range(2 * HB):
                sl = sq // 4 * 2 + sq % 2 + sq % 4 // 2 * HB
                fs = b_slice(sb, sl, 'hi', True) if sb.h else b_slice(sb, sl, 'lo', True) + ([] if not sb.early else b_slice(sb, sl, 'mi', True))
                fs = [((432.0 if sb.early else CH if sb.h else CL) / len(fs), f) for f in fs]
                if sq % 4 == 3:
                    fs = fs + [(320 / psp, lambda sq=sq, bs=bs: c_prep(sb, sq // 4, True, bs)) for bs in _spread(list(range(HB)), psp)]
                for j, (c_, f) in enumerate(fs):
                    out.append(((sq + j / len(fs)) / (2.0 * HB), c_, f))
        return (sorted(mx, key=lambda x: x[0]), sorted(out, key=lambda x: x[0]))

    def scheduler(wts, pieces, rpt, lag):
        cum = np.cumsum(wts) / np.sum(wts)
        slots = [[] for _ in wts]
        tot, run = (sum((c_ for _, c_, _ in pieces)), 0.0)
        for _, c_, f in pieces:
            slots[min(int(np.searchsorted(cum, run / tot, side='right')), len(wts) - 1)].append(f)
            run += c_
        pend, cnt, ran = ([], [0], [])
        keep = jnp.full((8, 128), zs[5], jnp.int32) == 0

        def call(f):
            if not any((f is g for g in ran)):
                ran.append(f)
                f()

        def need(fs):
            for f in fs:
                call(f)

        def tok(val):
            if not pieces:
                return val
            tiles = [val[r0:r0 + 8] for r0 in range(0, val.shape[0], 8)]
            for r0 in range(0, val.shape[0], rpt):
                due = [v for n, v in pend if n <= cnt[0]]
                pend[:] = [e for e in pend if e[0] > cnt[0]]
                for j, v in enumerate(due):
                    q = r0 // 8 + j % (rpt // 8)
                    tiles[q] = jnp.where(keep, tiles[q], v)
                dep['rv'], dep['out'] = (val[r0:r0 + 8], [])
                for f in slots[cnt[0]]:
                    call(f)
                pend.extend(((cnt[0] + lag, v) for _, v in dep['out'][::-1]))
                dep['rv'] = None
                cnt[0] += 1
            return jnp.concatenate(tiles, 0)
        return (tok, need)
    for s in range(NG + 2):
        if s != 1:
            wait(grp_copies(s % NG, s // NG))
        start(sched.get(s, []))
        if s == 0:
            wait(small[1:3])
            setup2()
        mx, pieces = conv_pieces(static_stage(s, 0), static_stage(s - 1, 1), static_stage(s - 2, 2), kq=KQ0, psp=PSP0)
        if s == 1:
            kvp = [f for e in mx for f in e[2]]
            bp = [e for e in pieces if not any((e[2] is f for f in kvp))]
            bp = bp[:int(len(bp) * BPRE)]
            for e in bp:
                e[2]()
            pieces = [e for e in pieces if not any((e is x for x in bp))]
            wait(grp_copies(1, 0))
        tok, need = scheduler([1.0] * (len(mx) * P // RPT0), pieces, RPT0, LAG0)
        for j, (_, f, pre) in enumerate(mx):
            need(pre)
            f(tok)

    npc = TM // PR

    def rows_of(i, r0=0, nr=TM):
        return pl.ds(pl.multiple_of(i * TM + r0, PR), nr)

    def a_layer_piece(r, i, iy, ps, stage_c):
        if not ps:
            return
        rr = rows_of(i, ps[0] * PR, len(ps) * PR)
        ry = rows_of(iy, ps[0] * PR, len(ps) * PR)
        x = r[rr, XC:XC + D].astype(f32)
        x = x + _ln(x) * y_v[ry, 0:D].astype(f32)
        r[rr, XC:XC + D] = x.astype(bf16)
        r[rr, stage_c:stage_c + D] = _ln(x).astype(bf16)

    def norm_piece(r, i, ps):
        if not ps:
            return
        rr = rows_of(i, ps[0] * PR, len(ps) * PR)
        r[rr, FH:F] = _ln(r[rr, FH:F].astype(f32)).astype(bf16)
    nzh = FH // TN
    noc = D // TN

    def z_chunk(r, i, c, tn=TN, tok=lambda v: v, ks=1, r0=0, nr=TM):
        cs = slice(c * tn, (c + 1) * tn)
        kk = D // ks
        acc = None
        for k in range(ks):
            part = _dot(_unpack(xnl[r0 // 2:(r0 + nr) // 2, k * kk:(k + 1) * kk]), win_v[k * kk:(k + 1) * kk, cs])
            if tn > 128 and ks > 1:
                part = jnp.concatenate([tok(part[:, 0:128]), part[:, 128:]], 1)
            else:
                part = tok(part)
            acc = part if acc is None else acc + part
        r[rows_of(i, r0, nr), cs] = _gelu(acc).astype(bf16)

    def g_chunk(r, i, c):
        cs = slice(c * TN, (c + 1) * TN)
        rr = rows_of(i)
        gg = _dot(wsp_v[rr, 0:S], r[0:S, FH + c * TN:FH + (c + 1) * TN])
        bb = bcol[rr, :]
        gg = gg + jnp.concatenate([bb] * (TN // 128), axis=1)
        ml[:, cs] = _pack((r[rr, cs].astype(f32) * gg).astype(bf16))

    def o_chunk(src, dst, dst_c, i, c, r0=0, nr=TM):
        cs = slice(c * TN, (c + 1) * TN)
        rr = rows_of(i, r0, nr)
        o = _dot(_unpack(ml[r0 // 2:(r0 + nr) // 2, 0:FH]), wout_v[:, cs])
        x = src[rr, XC + c * TN:XC + (c + 1) * TN].astype(f32) + o
        dst[rr, dst_c + c * TN:dst_c + (c + 1) * TN] = x.astype(bf16)
    parts_z = _spread(list(range(npc)), nzh)
    parts_o = _spread(list(range(npc)), noc)

    late = hi(4) + [q_copy(2)] + hi(5) + hi(6) + [q_copy(3)] + hi(7) + [q_copy(i) for i in range(4, NR)]
    q_copy(0).wait()
    for ps in parts_z:
        a_layer_piece(r1, 0, 0, ps, 0)
    wait(win_copy[:1])

    def ln_pieces(fn, lo=0.0, hi=1.0, n=LNP, sub=None):
        d = (hi - lo) / n
        return [(lo + j * d, lambda ps=ps: fn(ps)) for j, ps in enumerate(_spread(sub or list(range(npc)), n))]

    def p1_half(i, hh, lnp, conv=((), ()), first=False):
        mx, pieces = conv
        tn = TN1 if pieces else TNC
        nz1 = FH // tn
        ks = 2 * tn // 128
        rpt = TM // TPS
        grp = [[e for e in mx if min(int(e[0] * nz1 + 1e-06), nz1 - 1) == c] for c in range(nz1)]
        wts = []
        for c in range(nz1):
            for e in grp[c]:
                wts += [WC] * (P // rpt)
            wts += [1.0] * (TPS * (ks - 1)) + [W0] * TPS
        tok, need = scheduler(wts, pieces, rpt, LAG)
        for c in range(nz1):
            if first and c and (hh, c * tn // 128) in wpc:
                wpc[hh, c * tn // 128].wait()
                if hh == 1:
                    start(late[4:])
            for p_, f in lnp:
                if min(int(p_ * nz1 + 1e-06), nz1 - 1) == c:
                    f()
            for _, f, pre in grp[c]:
                need(pre)
                f(tok)
            z_chunk(r1, i, c + (nz1 if hh == 0 else 0), tn, tok, ks if pieces else 1)

    def p1a_body(i, carry, first):
        q_copy(i + 1).wait()
        wait(grp_copies(2 * i + 2, 1))
        base = i * PB

        def st(g0):
            sg = Stage(2 * i + g0, g0, 1, base)
            sg.early = first and g0 < MIG
            return sg
        xnl[:, 0:D] = _pack(r1[rows_of(i), 0:D])
        al = lambda ps: a_layer_piece(r1, i + 1, i + 1, ps, 0)
        h0, h1 = (list(range(npc // 2)), list(range(npc // 2, npc)))
        p1_half(i, 0, ln_pieces(al, n=LNH, sub=h0), conv_pieces(st(2), st(1), st(0)), first)
        wait(grp_copies(2 * i + 3, 1))
        if first:
            win_copy[1].wait()
            start(late[:4])
        p1_half(i, 1, ln_pieces(al, n=LNH, sub=h1), conv_pieces(st(3), st(2), st(1)), first)
        return carry
    p1a_body(zs[13], 0, True)
    jax.lax.fori_loop(1, 3, lambda i, cr: p1a_body(i, cr, False), 0)
    start([wsp_copy, wout_copy])
    wait([q_copy(i) for i in range(4, NR)])
    i3 = zs[8]
    xnl[:, 0:D] = _pack(r1[rows_of(i3), 0:D])
    b3 = zs[9]
    s14, s15 = (Stage(2 * i3, 0, 1, b3), Stage(2 * i3 + 1, 1, 1, b3))
    p1_half(i3, 0, [], conv_pieces(None, s15, s14))
    p1_half(i3, 1, ln_pieces(lambda ps: a_layer_piece(r1, i3 + 1, i3 + 1, ps, 0), A4L, 1.0, A4N), conv_pieces(None, None, s15, A4F))

    def p1c_body(i, carry):
        iy = jnp.minimum(i + 1, NR - 1)
        xnl[:, 0:D] = _pack(r1[rows_of(i), 0:D])
        p1_half(i, 0, ln_pieces(lambda ps: a_layer_piece(r1, i + 1, iy, ps, 0)))
        for c in range(2 * nzh):
            norm_piece(r1, i if c % 2 else i - 4, parts_z[c // 2])
            z_chunk(r1, i, c // 2, r0=c % 2 * (TM // 2), nr=TM // 2)
        return carry
    jax.lax.fori_loop(4, NR, p1c_body, 0)

    wsp_copy.wait()
    wout_copy.wait()
    last = NR - 1
    for c in range(nzh):
        g_chunk(r1, 0, c)
    np1 = ORS // PR
    for c in range(noc):
        o_chunk(r1, r2, XC, 0, c, 0, ORS)
    for c, ps in enumerate(_spread(list(range(np1)), noc)):
        a_layer_piece(r2, zs[13], zs[13], ps, FH)
        o_chunk(r1, r2, XC, 0, c, ORS, TM - ORS)
    for ps in _spread(list(range(np1, npc)), 4):
        a_layer_piece(r2, 0, 0, ps, FH)

    def p2_body(i, carry):
        xnl[:, 0:D] = _pack(r2[rows_of(i - 1), FH:FH + D])
        for c in range(nzh):
            g_chunk(r1, i, c)
        for c in range(nzh):
            z_chunk(r2, i - 1, nzh + c)
        pn = _spread(list(range(npc)), 2 * noc)
        for c in range(2 * noc):
            norm_piece(r2, i - 1, pn[c])
            o_chunk(r1, r2, XC, i, c % noc, c // noc * (TM // 2), TM // 2)
        for c in range(nzh):
            a_layer_piece(r2, i, i, parts_z[c], FH)
            z_chunk(r2, i - 1, c)
        return carry
    jax.lax.fori_loop(1, NR, p2_body, 0)
    xnl[:, 0:D] = _pack(r2[rows_of(last), FH:FH + D])
    for c in range(nzh):
        z_chunk(r2, last, nzh + c)
    for c in range(nzh):
        norm_piece(r2, last, parts_z[c])
        z_chunk(r2, last, c)

    for c in range(nzh):
        g_chunk(r2, 0, c)

    def p3_body(i, carry):
        for c in range(noc):
            o_chunk(r2, y_v, 0, i - 1, c)
        out_copy(i - 1).start()
        for c in range(nzh):
            g_chunk(r2, i, c)
        return carry
    jax.lax.fori_loop(0, 3, lambda j, cr: p3_body(2 * j + 2, p3_body(2 * j + 1, cr)), 0)
    p3_body(NR - 1, 0)

    def out_last(c):
        cs = slice(c * TN, (c + 1) * TN)
        return pltpu.make_async_copy(y_v.at[blk(last), cs], out_hbm.at[0, blk(last), cs], sem_o.at[NR + c])
    for c in range(noc):
        o_chunk(r2, y_v, 0, NR - 1, c)
        out_last(c).start()
    for i in range(NR - OSP):
        out_copy(i).wait()
    wait([out_last(c) for c in range(noc)])

@jax.jit
def pallas_interleave_layers__ssm_conv_h3__mixer_gmlp__prompt_kernel(A_q, A_k, A_v, A_shift_k, A_ssm_k, A_ssm_D, B_x, B_w_in, B_w_sp, B_b_sp, B_w_out):
    del B_x
    anyspec = pl.BlockSpec(memory_space=pl.ANY)
    return pl.pallas_call(_kernel, grid=(1,), in_specs=[anyspec] * 11, out_specs=anyspec, out_shape=jax.ShapeDtypeStruct((1, S, D), bf16), scratch_shapes=[pltpu.VMEM((D, F), bf16), pltpu.VMEM((S, S), bf16), pltpu.VMEM((FH, D + PS2), bf16), pltpu.VMEM((S, D), bf16), pltpu.VMEM((S + TM, RW), bf16), pltpu.VMEM((S + 16, RW), bf16), pltpu.VMEM((TM // 2, D), u32), pltpu.VMEM((TM // 2, FH), u32), pltpu.VMEM((NTW, P + PADW, 128), u32), pltpu.VMEM((96, P + PADW, 128), u32), pltpu.VMEM((HS // 2, 128), u32), pltpu.VMEM((HS // 2, 128), u32), pltpu.VMEM((HS // 2, 128), u32), pltpu.VMEM((NG, HS // 2, 128), u32), pltpu.VMEM((2 * HB, P + PADW, 128), u32), pltpu.VMEM((HS + 8, 128), f32), pltpu.VMEM((3 * P // 2, 128), u32), pltpu.VMEM((S, 128), f32), pltpu.VMEM((NG, 8, 128), f32), pltpu.SMEM((16,), jnp.int32), pltpu.VMEM((4, D), bf16), pltpu.VMEM((D,), bf16), pltpu.VMEM((S,), bf16), pltpu.VMEM((3 * P, 128), bf16), pltpu.SemaphoreType.DMA((2 * NG,)), pltpu.SemaphoreType.DMA((2 * NG,)), pltpu.SemaphoreType.DMA((2 * NG,)), pltpu.SemaphoreType.DMA((16,)), pltpu.SemaphoreType.DMA((NR,)), pltpu.SemaphoreType.DMA((NR + 4,)), pltpu.SemaphoreType.DMA((7,))], compiler_params=pltpu.CompilerParams(dimension_semantics=('arbitrary',), vmem_limit_bytes=124 * 1024 * 1024))(A_q, A_k, A_v, A_shift_k.T, A_ssm_k, A_ssm_D, B_w_in, B_w_sp, B_b_sp, B_w_out, _dft_constants())
```
